```python
import os as _os
_os.environ.setdefault('JAX_PLATFORMS', 'cpu')
import jax
import jax.numpy as jnp

def _softmax(x, axis=-1):
    return jax.nn.softmax(x, axis=axis)

def _gelu(x):
    return jax.nn.gelu(x, approximate=True)

def _silu(x):
    return jax.nn.silu(x)

def _sigmoid(x):
    return jax.nn.sigmoid(x)

def _layernorm(x, axis=-1, eps=1e-05):
    m = jnp.mean(x, axis=axis, keepdims=True)
    v = jnp.var(x, axis=axis, keepdims=True)
    return (x - m) / jnp.sqrt(v + eps)

def _scatter_add(tgt, idx, src, axis=0):
    return tgt.at[idx].add(src)

def _segment_sum(src, seg, n):
    return jax.ops.segment_sum(src, seg, n)

class _Rng:

    def __init__(self, key):
        self._k = key

    def _next(self):
        self._k, sub = jax.random.split(self._k)
        return sub

    def normal(self, shape):
        return jax.random.normal(self._next(), shape, dtype=jnp.bfloat16)

    def randint(self, lo, hi, shape):
        return jax.random.randint(self._next(), shape, lo, hi, dtype=jnp.int32)

    def uniform(self, shape, lo=0.0, hi=1.0):
        return jax.random.uniform(self._next(), shape, jnp.bfloat16, lo, hi)

    def permutation(self, n):
        return jax.random.permutation(self._next(), n)
kernel_name = 'adaLN_cond__softmax_full_mha__mixer_gmlp__prompt'

def setup_inputs():
    _rng = _Rng(jax.random.key(int.from_bytes(__import__("os").urandom(4), "little")))
    _w = lambda a: (lambda t: t.astype(jnp.bfloat16) if jnp.issubdtype(t.dtype, jnp.floating) else t)(jnp.asarray(a))

    def _A_setup():
        B, S, D = (1, 2048, 512)
        return {'x': _w((lambda *s: _rng.normal(s) * 0.05)(B, S, D)), 'wqkv': _w((lambda *s: _rng.normal(s) * 0.05)(D, 3 * D)), 'wo': _w((lambda *s: _rng.normal(s) * 0.05)(D, D))}
    _A_in = _A_setup()

    def _B_setup():
        B, S, D, F = (1, 2048, 512, 1792)
        Fh = F // 2
        return {'x': _w((lambda *s: _rng.normal(s) * 0.05)(B, S, D)), 'w_in': _w((lambda *s: _rng.normal(s) * 0.4)(D, 2 * Fh)), 'w_sp': _w(0.01 * (lambda *s: _rng.normal(s) * 0.4)(S, S)), 'b_sp': _w(1.0 + 0.01 * (lambda *s: _rng.normal(s) * 0.05)(S)), 'w_out': _w((lambda *s: _rng.normal(s) * 0.05)(Fh, D))}
    _B_in = _B_setup()
    return {'A_x': _A_in['x'], 'A_wqkv': _A_in['wqkv'], 'A_wo': _A_in['wo'], 'B_x': _B_in['x'], 'B_w_in': _B_in['w_in'], 'B_w_sp': _B_in['w_sp'], 'B_b_sp': _B_in['b_sp'], 'B_w_out': _B_in['w_out'], 'c': _w((lambda *s: _rng.normal(s) * 0.05)(1, 512) * 8.0), 'w_mod': _w((lambda *s: _rng.normal(s) * 0.05)(512, 6 * 512) * 512 ** (-0.5) * 8.0)}

def reference(A_x, A_wqkv, A_wo, B_x, B_w_in, B_w_sp, B_b_sp, B_w_out, c, w_mod):

    def _A_ref(x, wqkv, wo):
        B, S, D = x.shape
        H = 32
        Dh = D // H
        qkv = (lambda x, *d: x.transpose(*d))((x @ wqkv).reshape(B, S, 3, H, Dh), 2, 0, 3, 1, 4)
        q, k, v = (qkv[0], qkv[1], qkv[2])
        scale = Dh ** (-0.5)
        scores = jnp.einsum('bhqd,bhkd->bhqk', q, k) * scale
        p = _softmax(scores, axis=-1)
        o = jnp.einsum('bhqk,bhkd->bhqd', p, v)
        return (lambda x, *d: x.transpose(*d))(o, 0, 2, 1, 3).reshape(B, S, D) @ wo

    def _B_ref(x, w_in, w_sp, b_sp, w_out):
        B, S, D = x.shape
        F = w_in.shape[-1]
        Fh = F // 2
        z = _gelu(jnp.einsum('bsd,df->bsf', x, w_in))
        z1 = z[..., :Fh].copy()
        z2 = _layernorm(z[..., Fh:], axis=-1)
        g = jnp.einsum('ts,bsf->btf', w_sp, z2) + b_sp[None, :, None]
        return jnp.einsum('bsf,fd->bsd', z1 * g, w_out)
    x = A_x
    mod = (_silu(c) @ w_mod).reshape(c.shape[0], 6, 1, -1)
    sa, ca, ga, sb, cb, gb = (mod[:, 0].copy(), mod[:, 1].copy(), mod[:, 2].copy(), mod[:, 3].copy(), mod[:, 4].copy(), mod[:, 5].copy())
    h = _layernorm(x, axis=-1) * (1 + ca) + sa
    x = x + ga * _A_ref(h, A_wqkv, A_wo)
    h = _layernorm(x, axis=-1) * (1 + cb) + sb
    x = x + gb * _B_ref(h, B_w_in, B_w_sp, B_b_sp, B_w_out)
    return x
```

```python
import functools
import math

import jax
import jax.numpy as jnp
from jax import lax
import jax.experimental.pallas as pl
import jax.experimental.pallas.tpu as pltpu

S = 2048
D = 512
H = 32
DH = 16
F = 1792
FH = 896
EPS = 1e-5
bf16 = jnp.bfloat16
f32 = jnp.float32

TQ = 512
TK = 128
NSUB = 2
NQ = S // TQ
NB = H * NQ
NS = NB // NSUB
TA = 256
TC = 256
TD = 256
QSCALE = (DH ** -0.5) * math.log2(math.e)
NT = (((1,), (1,)), ((), ()))
TN = (((0,), (0,)), ((), ()))


def _ln(x):
    m = jnp.mean(x, axis=-1, keepdims=True)
    xc = x - m
    v = jnp.mean(xc * xc, axis=-1, keepdims=True)
    return xc * lax.rsqrt(v + EPS)


def _gelu(x):
    c = math.sqrt(2.0 / math.pi)
    return 0.5 * x * (1.0 + jnp.tanh(c * (x + 0.044715 * (x * x * x))))


def _kernel(x_hbm, wqkv_hbm, wo_hbm, win_hbm, wsp_hbm, bsp_hbm, wout_hbm, c_hbm, wmod_hbm,
            out_hbm,
            x_v, wqkv_v, wo_v, win_v, wsp_v, bsp_v, wout_v, c_v, wmod_v,
            wqT_v, wvT_v, k_v, qT_v, vT_v, oT_v, s0, s1, x1_v, z1_v, z2_v, bcol_v, mod_v, out_v,
            sems, osems, *, phases):
    cp = {}
    def mk(name, src, dst, i):
        cp[name] = pltpu.make_async_copy(src, dst, sems.at[i])
    mk("c", c_hbm, c_v, 0)
    mk("wmod0", wmod_hbm.at[:, 0:2 * D], wmod_v.at[:, 0:2 * D], 1)
    mk("x", x_hbm, x_v, 2)
    mk("wqkv", wqkv_hbm, wqkv_v, 3)
    mk("wmod1", wmod_hbm.at[:, 2 * D:6 * D], wmod_v.at[:, 2 * D:6 * D], 4)
    mk("wo", wo_hbm, wo_v, 5)
    mk("win", win_hbm, win_v, 6)
    mk("bsp", bsp_hbm, bsp_v, 7)
    mk("wsp", wsp_hbm, wsp_v, 8)
    mk("wout", wout_hbm, wout_v, 9)
    for n in ("c", "wmod0", "wqkv", "x"):
        cp[n].start()

    cp["c"].wait()
    cf = c_v[...].astype(f32)
    sc = (cf * jax.nn.sigmoid(cf)).astype(bf16)
    sc8 = jnp.broadcast_to(sc, (8, D))
    cp["wmod0"].wait()
    mod_v[:, 0:2 * D] = jnp.dot(sc8, wmod_v[:, 0:2 * D], preferred_element_type=f32)
    cp["wqkv"].wait()
    wqT_v[...] = wqkv_v[:, 0:D].astype(f32).T.astype(bf16)
    wvT_v[...] = wqkv_v[:, 2 * D:3 * D].astype(f32).T.astype(bf16)
    cp["x"].wait()
    for n in ("wmod1", "wo", "win", "bsp", "wsp", "wout"):
        cp[n].start()

    def phase_a(i, carry):
        r = pl.multiple_of(i * TA, TA)
        xt = x_v[pl.ds(r, TA), :].astype(f32)
        h = (_ln(xt) * (1.0 + mod_v[0:1, D:2 * D]) + mod_v[0:1, 0:D]).astype(bf16)
        k_v[pl.ds(r, TA), :] = jnp.dot(h, wqkv_v[:, D:2 * D], preferred_element_type=f32).astype(bf16)
        qT = lax.dot_general(wqT_v[...], h, NT, preferred_element_type=f32)
        qT_v[:, pl.ds(r, TA)] = (qT * QSCALE).astype(bf16)
        vT = lax.dot_general(wvT_v[...], h, NT, preferred_element_type=f32)
        vT_v[:, pl.ds(r, TA)] = vT.astype(bf16)
        return carry
    if "A" in phases:
        lax.fori_loop(0, S // TA, phase_a, 0)

    row = lax.broadcasted_iota(jnp.int32, (128, TQ), 0) // DH

    def step(t, m_curs, s_rd, s_wr, produce=True, consume=True):
        outs = []
        for u in range(NSUB):
            b = t * NSUB + u
            if produce:
                bn = b + NSUB
                hn = bn // NQ
                gl = pl.multiple_of((hn // 8) * 128, 128)
                qg = qT_v[pl.ds(gl, 128), pl.ds(pl.multiple_of((bn % NQ) * TQ, TQ), TQ)]
                qw = jnp.where(row == hn % 8, qg, jnp.zeros_like(qg))
            if consume:
                hr = pl.multiple_of((b // NQ) * DH, DH)
                qc = pl.multiple_of((b % NQ) * TQ, TQ)
                m_cur = m_curs[u]
            mx = jnp.full((8, TQ), -jnp.inf, f32)
            l = jnp.zeros((8, TQ), f32)
            acc = jnp.zeros((DH, TQ), f32)
            for c in range(S // TK):
                if produce:
                    sn = jnp.dot(k_v[c * TK:(c + 1) * TK, pl.ds(gl, 128)], qw, preferred_element_type=f32)
                    s_wr[u, c * TK:(c + 1) * TK, :] = sn
                    mx = jnp.maximum(mx, sn.reshape(TK // 8, 8, TQ).max(axis=0))
                if consume:
                    p = jnp.exp2(s_rd[u, c * TK:(c + 1) * TK, :] - m_cur)
                    for r in reversed(range(TK // 16)):
                        l = l + (p[r * 16 + 8:r * 16 + 16] + p[r * 16:r * 16 + 8])
                    acc = acc + jnp.dot(vT_v[pl.ds(hr, DH), c * TK:(c + 1) * TK], p.astype(bf16),
                                        preferred_element_type=f32)
            if consume:
                o = acc / l.sum(axis=0, keepdims=True)
                oT_v[pl.ds(hr, DH), pl.ds(qc, TQ)] = o.astype(bf16)
            outs.append(mx.max(axis=0, keepdims=True))
        return tuple(outs)

    if "B" in phases:
        m0 = step(-1, None, None, s0, consume=False)

        def body(t, m):
            return lax.cond(t % 2 == 0, lambda m: step(t, m, s0, s1), lambda m: step(t, m, s1, s0), m)
        m = lax.fori_loop(0, NS - 1, body, m0)
        step(NS - 1, m, s1 if (NS - 1) % 2 else s0, None, produce=False)

    cp["wmod1"].wait()
    mod_v[:, 2 * D:6 * D] = jnp.dot(sc8, wmod_v[:, 2 * D:6 * D], preferred_element_type=f32)
    cp["bsp"].wait()
    for j in range(S // 128):
        bj = jnp.broadcast_to(bsp_v[:, j * 128:(j + 1) * 128].astype(f32), (128, 128))
        bcol_v[j * 128:(j + 1) * 128, :] = bj.T
    cp["wo"].wait()
    cp["win"].wait()

    def phase_c(i, carry):
        r = pl.multiple_of(i * TC, TC)
        y = lax.dot_general(oT_v[:, pl.ds(r, TC)], wo_v[...], TN, preferred_element_type=f32)
        x1 = x_v[pl.ds(r, TC), :].astype(f32) + mod_v[0:1, 2 * D:3 * D] * y
        x1_v[pl.ds(r, TC), :] = x1
        h2 = (_ln(x1) * (1.0 + mod_v[0:1, 4 * D:5 * D]) + mod_v[0:1, 3 * D:4 * D]).astype(bf16)
        z1 = _gelu(jnp.dot(h2, win_v[:, 0:FH], preferred_element_type=f32))
        z1_v[pl.ds(r, TC), :] = z1.astype(bf16)
        z2 = _gelu(jnp.dot(h2, win_v[:, FH:F], preferred_element_type=f32))
        z2_v[pl.ds(r, TC), :] = _ln(z2).astype(bf16)
        return carry
    if "C" in phases:
        lax.fori_loop(0, S // TC, phase_c, 0)

    cp["wsp"].wait()
    cp["wout"].wait()

    def out_copy(i):
        r = pl.multiple_of(i * TD, TD)
        return pltpu.make_async_copy(out_v.at[pl.ds(r, TD), :], out_hbm.at[pl.ds(r, TD), :], osems.at[i])

    def phase_d(i, carry):
        r = pl.multiple_of(i * TD, TD)
        if "D" in phases:
            g = jnp.dot(wsp_v[pl.ds(r, TD), :], z2_v[...], preferred_element_type=f32)
            bc = bcol_v[pl.ds(r, TD), :]
            g = g + jnp.concatenate([bc] * (FH // 128), axis=1)
            u = (z1_v[pl.ds(r, TD), :].astype(f32) * g).astype(bf16)
            y2 = jnp.dot(u, wout_v[...], preferred_element_type=f32)
            out_v[pl.ds(r, TD), :] = (x1_v[pl.ds(r, TD), :] + mod_v[0:1, 5 * D:6 * D] * y2).astype(bf16)
        else:
            out_v[pl.ds(r, TD), :] = x_v[pl.ds(r, TD), :]
        out_copy(i).start()
        return carry
    lax.fori_loop(0, S // TD, phase_d, 0)
    for i in range(S // TD):
        out_copy(i).wait()


def make(phases="ABCD"):
    @jax.jit
    def fn(A_x, A_wqkv, A_wo, B_x, B_w_in, B_w_sp, B_b_sp, B_w_out, c, w_mod):
        x = A_x.reshape(S, D)
        bsp = B_b_sp.reshape(1, S)
        any_spec = pl.BlockSpec(memory_space=pl.ANY)
        out = pl.pallas_call(
            functools.partial(_kernel, phases=phases),
            out_shape=jax.ShapeDtypeStruct((S, D), bf16),
            in_specs=[any_spec] * 9,
            out_specs=any_spec,
            scratch_shapes=[
                pltpu.VMEM((S, D), bf16),
                pltpu.VMEM((D, 3 * D), bf16),
                pltpu.VMEM((D, D), bf16),
                pltpu.VMEM((D, F), bf16),
                pltpu.VMEM((S, S), bf16),
                pltpu.VMEM((1, S), bf16),
                pltpu.VMEM((FH, D), bf16),
                pltpu.VMEM((1, D), bf16),
                pltpu.VMEM((D, 6 * D), bf16),
                pltpu.VMEM((D, D), bf16),
                pltpu.VMEM((D, D), bf16),
                pltpu.VMEM((S, D), bf16),
                pltpu.VMEM((D, S), bf16),
                pltpu.VMEM((D, S), bf16),
                pltpu.VMEM((D, S), bf16),
                pltpu.VMEM((NSUB, S, TQ), f32),
                pltpu.VMEM((NSUB, S, TQ), f32),
                pltpu.VMEM((S, D), f32),
                pltpu.VMEM((S, FH), bf16),
                pltpu.VMEM((S, FH), bf16),
                pltpu.VMEM((S, 128), f32),
                pltpu.VMEM((8, 6 * D), f32),
                pltpu.VMEM((S, D), bf16),
                pltpu.SemaphoreType.DMA((10,)),
                pltpu.SemaphoreType.DMA((S // TD,)),
            ],
            compiler_params=pltpu.CompilerParams(vmem_limit_bytes=110 * 2 ** 20),
        )(x, A_wqkv, A_wo, B_w_in, B_w_sp, bsp, B_w_out, c, w_mod)
        return out.reshape(1, S, D)
    return fn


pallas_adaLN_cond__softmax_full_mha__mixer_gmlp__prompt_kernel = make()
```

```python
import functools
import math

import jax
import jax.numpy as jnp
from jax import lax
import jax.experimental.pallas as pl
import jax.experimental.pallas.tpu as pltpu

S = 2048
D = 512
H = 32
DH = 16
F = 1792
FH = 896
EPS = 1e-5
bf16 = jnp.bfloat16
f32 = jnp.float32
u32 = jnp.uint32

TQ = 128
TK = 128
NQ = S // TQ
NC = S // TK
VR = 16
SV = VR * NC
NL = 4
TF = 256
TA = 256
TC = 256
TD = 256
QSCALE = (DH ** -0.5) * math.log2(math.e)
L_LO = 2.0 ** -80
L_HI = 2.0 ** 100
F_MAX = 3.0e38
NT = (((1,), (1,)), ((), ()))
TN = (((0,), (0,)), ((), ()))


def _ln(x):
    m = jnp.mean(x, axis=-1, keepdims=True)
    xc = x - m
    v = jnp.mean(xc * xc, axis=-1, keepdims=True)
    return xc * lax.rsqrt(v + EPS)


def _gelu(x):
    c = math.sqrt(2.0 / math.pi)
    return 0.5 * x * (1.0 + jnp.tanh(c * (x + 0.044715 * (x * x * x))))


def _pack_rows(p):
    return jnp.concatenate(
        [pltpu.pack_elementwise([p[r * 16:r * 16 + 8], p[r * 16 + 8:r * 16 + 16]], packed_dtype=bf16)
         for r in range(p.shape[0] // 16)], axis=0)


def _kernel(x_hbm, wqkv_hbm, wo_hbm, win_hbm, wsp_hbm, bsp_hbm, wout_hbm, c_hbm, wmod_hbm,
            out_hbm,
            x_v, wqkv_v, wo_v, win_v, wsp_v, wout_v, wmod_v,
            wqT_v, wvT_v, k_v, kf_v, qT_v, qf_v, vT_v, oT_v,
            kb0, kb1, kr0, kr1, p0, p1, l0, l1, bad_v, sf_v,
            x1_v, z1_v, z2_v, bcol_v, mod_v, out_v, bsp_v, c_v, pad_v,
            sems, osems, *, phases):
    cp = {}
    def mk(name, src, dst, i):
        cp[name] = pltpu.make_async_copy(src, dst, sems.at[i])
    mk("c", c_hbm, c_v, 0)
    mk("wmod0", wmod_hbm.at[:, 0:2 * D], wmod_v.at[:, 0:2 * D], 1)
    mk("x", x_hbm, x_v, 2)
    mk("wqkv", wqkv_hbm, wqkv_v, 3)
    mk("wmod1", wmod_hbm.at[:, 2 * D:6 * D], wmod_v.at[:, 2 * D:6 * D], 4)
    mk("wo", wo_hbm, wo_v, 5)
    mk("win", win_hbm, win_v, 6)
    mk("bsp", bsp_hbm, bsp_v, 7)
    mk("wsp", wsp_hbm, wsp_v, 8)
    mk("wout", wout_hbm, wout_v, 9)
    for n in ("c", "wmod0", "wqkv", "x"):
        cp[n].start()

    cp["c"].wait()
    cf = c_v[...].astype(f32)
    sc = (cf * jax.nn.sigmoid(cf)).astype(bf16)
    sc8 = jnp.broadcast_to(sc, (8, D))
    cp["wmod0"].wait()
    mod_v[:, 0:2 * D] = jnp.dot(sc8, wmod_v[:, 0:2 * D], preferred_element_type=f32)
    cp["wqkv"].wait()
    wqT_v[...] = wqkv_v[:, 0:D].astype(f32).T.astype(bf16)
    wvT_v[...] = wqkv_v[:, 2 * D:3 * D].astype(f32).T.astype(bf16)
    cp["x"].wait()
    for n in ("wmod1", "wo", "win", "bsp", "wsp", "wout"):
        cp[n].start()

    def a_ln(i):
        r = pl.multiple_of(i * TA, TA)
        xt = x_v[pl.ds(r, TA), :].astype(f32)
        hf = _ln(xt) * (1.0 + mod_v[0:1, D:2 * D]) + mod_v[0:1, 0:D]
        return hf.astype(bf16), pltpu.bitcast(_pack_rows(hf), bf16)

    def a_mm(i, hs):
        h, hp = hs
        r = pl.multiple_of(i * TA, TA)
        kk = jnp.dot(h, wqkv_v[:, D:2 * D], preferred_element_type=f32)
        k_v[pl.ds(pl.multiple_of(i * (TA // 2), TA // 2), TA // 2), :] = pltpu.bitcast(kk.astype(bf16), u32)
        for j in range(TA // TK):
            kf_v[pl.ds(pl.multiple_of((i * (TA // TK) + j) * VR, VR), VR), :] = kk[(j + 1) * TK - VR:(j + 1) * TK]
        qT = lax.dot_general(wqT_v[...], h, NT, preferred_element_type=f32) * QSCALE
        qf_v[:, :, pl.ds(r, TA)] = qT.reshape(H, DH, TA)
        qT_v[:, :, pl.ds(r, TA)] = qT.astype(bf16).reshape(H, DH, TA)
        vT = lax.dot_general(wvT_v[...], hp, NT, preferred_element_type=f32)
        vT_v[:, :, pl.ds(r, TA)] = vT.astype(bf16).reshape(H, DH, TA)

    for _ in range(phases.count("A")):
        def phase_a(i, hs):
            hn = a_ln(i + 1)
            a_mm(i, hs)
            return hn
        hs = lax.fori_loop(0, S // TA - 1, phase_a, a_ln(0))
        a_mm(S // TA - 1, hs)

    def build_k(h, kb, kr, do_kb=True):
        gl = pl.multiple_of((h // 8) * 128, 128)
        sh = (128 - (h % 8) * DH) % 128
        kr[...] = pltpu.roll(k_v[:, pl.ds(gl, 128)], sh, 1)
        if do_kb:
            kk = pltpu.roll(kf_v[:, pl.ds(gl, 128)], sh, 1)
            for d in range(DH):
                kb[d] = jnp.broadcast_to(kk[:, d:d + 1], (SV, 128))

    def block(u, hp, hc, p_rd, p_wr, l_rd, l_wr, kb_rd, kr_rd, vr, bad):
        produce = hp is not None
        consume = hc is not None
        q0 = u * TQ
        if produce:
            qw = qT_v[hp, :, q0:q0 + TQ]
        l = [None] * NL
        acc = None
        for c in range(NC):
            if produce:
                parts = []
                if vr:
                    a0 = a1 = None
                    for d in range(DH):
                        qb = jnp.broadcast_to(qf_v[hp, d:d + 1, q0:q0 + TQ], (8, TQ))
                        t0 = kb_rd[d, c * VR:c * VR + 8, :] * qb
                        t1 = kb_rd[d, c * VR + 8:c * VR + 16, :] * qb
                        a0 = t0 if a0 is None else a0 + t0
                        a1 = t1 if a1 is None else a1 + t1
                    e0 = jnp.exp2(a0)
                    e1 = jnp.exp2(a1)
                    parts.append(e0 + e1)
                    r0 = ((c + 1) * TK - VR) // 2
                    p_wr[u, r0:r0 + 8, :] = pltpu.pack_elementwise([e0, e1], packed_dtype=bf16)
                st = c * TK
                sz = TK - vr
                kk = pltpu.bitcast(kr_rd[st // 2:(st + sz) // 2, :], bf16)[:, 0:DH]
                p = jnp.exp2(jnp.dot(kk, qw, preferred_element_type=f32))
                for r in range(sz // 16):
                    parts.append(p[r * 16:r * 16 + 8] + p[r * 16 + 8:r * 16 + 16])
                for v in parts:
                    l[c % NL] = v if l[c % NL] is None else l[c % NL] + v
                for r in range(sz // 16):
                    p_wr[u, st // 2 + r * 8:st // 2 + r * 8 + 8, :] = pltpu.pack_elementwise(
                        [p[r * 16:r * 16 + 8], p[r * 16 + 8:r * 16 + 16]], packed_dtype=bf16)
            if consume:
                pb = pltpu.bitcast(p_rd[u, c * TK // 2:(c + 1) * TK // 2, :], bf16)
                t = jnp.dot(vT_v[hc, :, c * TK:(c + 1) * TK], pb, preferred_element_type=f32)
                acc = t if acc is None else acc + t
        if consume:
            ls = l_rd[:, q0:q0 + TQ].sum(axis=0, keepdims=True)
            oT_v[pl.ds(pl.multiple_of(hc * DH, DH), DH), q0:q0 + TQ] = (acc * (1.0 / ls)).astype(bf16)
            aa = jnp.abs(acc)
            ok = (aa[0:8] <= F_MAX) & (aa[8:16] <= F_MAX) & (ls >= L_LO) & (ls <= L_HI)
            bad = jnp.where(ok, bad, 1.0)
        if produce:
            l_wr[:, q0:q0 + TQ] = (l[0] + l[1]) + (l[2] + l[3])
        return bad

    def step(h, p_rd, p_wr, l_rd, l_wr, kb_rd, kr_rd, kb_wr, kr_wr, produce=True, consume=True, vr=VR):
        bad = bad_v[...] if consume else None
        for u in range(NQ):
            bad = block(u, h + 1 if produce else None, h if consume else None,
                        p_rd, p_wr, l_rd, l_wr, kb_rd, kr_rd, vr, bad)
        if consume:
            bad_v[...] = bad
        if produce:
            build_k(jnp.minimum(h + 2, H - 1), kb_wr, kr_wr)

    bad_v[...] = jnp.zeros((8, TQ), f32)
    if "B" in phases:
        build_k(0, kb0, kr0, do_kb=False)
        step(-1, None, p0, None, l0, kb0, kr0, kb1, kr1, consume=False, vr=0)

        def body(h, carry):
            lax.cond(h % 2 == 0,
                     lambda: step(h, p0, p1, l0, l1, kb1, kr1, kb0, kr0),
                     lambda: step(h, p1, p0, l1, l0, kb0, kr0, kb1, kr1))
            return carry
        lax.fori_loop(0, (15 if 'h' in phases else H - 1), body, 0)
        step(H - 1, p1, None, l1, None, None, None, None, None, produce=False)

    def fallback():
        row = lax.broadcasted_iota(jnp.int32, (128, TF), 0) // DH

        def fb(b, carry):
            h = b // (S // TF)
            q0 = pl.multiple_of((b % (S // TF)) * TF, TF)
            g = h // 8
            gl = pl.multiple_of(g * 128, 128)
            qg = qf_v[pl.ds(g * 8, 8), :, pl.ds(q0, TF)].reshape(128, TF)
            qw = jnp.where(row == h % 8, qg, 0.0).astype(bf16)
            mx = jnp.full((8, TF), -jnp.inf, f32)
            for c in range(NC):
                kk = pltpu.bitcast(k_v[c * TK // 2:(c + 1) * TK // 2, pl.ds(gl, 128)], bf16)
                s = jnp.dot(kk, qw, preferred_element_type=f32)
                sf_v[c * TK:(c + 1) * TK, :] = s
                mx = jnp.maximum(mx, s.reshape(TK // 8, 8, TF).max(axis=0))
            m = mx.max(axis=0, keepdims=True)
            l = jnp.zeros((8, TF), f32)
            acc = jnp.zeros((DH, TF), f32)
            for c in range(NC):
                p = jnp.exp2(sf_v[c * TK:(c + 1) * TK, :] - m)
                l = l + p.reshape(TK // 8, 8, TF).sum(axis=0)
                acc = acc + jnp.dot(vT_v[h, :, c * TK:(c + 1) * TK], pltpu.bitcast(_pack_rows(p), bf16),
                                    preferred_element_type=f32)
            o = acc / l.sum(axis=0, keepdims=True)
            oT_v[pl.ds(pl.multiple_of(h * DH, DH), DH), pl.ds(q0, TF)] = o.astype(bf16)
            return carry
        lax.fori_loop(0, H * (S // TF), fb, 0)

    if "F" in phases:
        fallback()
    elif "N" not in phases:
        pl.when(jnp.max(bad_v[...]) > 0.0)(fallback)

    cp["wmod1"].wait()
    mod_v[:, 2 * D:6 * D] = jnp.dot(sc8, wmod_v[:, 2 * D:6 * D], preferred_element_type=f32)
    cp["bsp"].wait()
    for j in range(S // 128):
        bj = jnp.broadcast_to(bsp_v[:, j * 128:(j + 1) * 128].astype(f32), (128, 128))
        bcol_v[j * 128:(j + 1) * 128, :] = bj.T
    cp["wo"].wait()
    cp["win"].wait()

    def c_s1(i):
        r = pl.multiple_of(i * TC, TC)
        y = lax.dot_general(oT_v[:, pl.ds(r, TC)], wo_v[...], TN, preferred_element_type=f32)
        x1 = x_v[pl.ds(r, TC), :].astype(f32) + mod_v[0:1, 2 * D:3 * D] * y
        x1_v[pl.ds(r, TC), :] = x1
        return (_ln(x1) * (1.0 + mod_v[0:1, 4 * D:5 * D]) + mod_v[0:1, 3 * D:4 * D]).astype(bf16)

    def c_z2(i, h2):
        r = pl.multiple_of(i * TC, TC)
        z2 = _gelu(jnp.dot(h2, win_v[:, FH:F], preferred_element_type=f32))
        z2_v[pl.ds(r, TC), :] = _ln(z2).astype(bf16)

    def c_z1(i, h2):
        r = pl.multiple_of(i * TC, TC)
        z1 = _gelu(jnp.dot(h2, win_v[:, 0:FH], preferred_element_type=f32))
        z1_v[pl.ds(r, TC), :] = z1.astype(bf16)

    for _ in range(phases.count("C")):
        def phase_c(i, h2):
            c_z2(i, h2)
            hn = c_s1(i + 1)
            c_z1(i, h2)
            return hn
        h2 = lax.fori_loop(0, S // TC - 1, phase_c, c_s1(0))
        c_z2(S // TC - 1, h2)
        c_z1(S // TC - 1, h2)

    cp["wsp"].wait()
    cp["wout"].wait()

    def out_copy(i):
        r = pl.multiple_of(i * TD, TD)
        return pltpu.make_async_copy(out_v.at[pl.ds(r, TD), :], out_hbm.at[pl.ds(r, TD), :], osems.at[i])

    nd = max(1, phases.count("D"))
    def phase_d(ii, carry):
        i = ii % (S // TD)
        r = pl.multiple_of(i * TD, TD)
        if "D" in phases:
            g = jnp.dot(wsp_v[pl.ds(r, TD), :], z2_v[...], preferred_element_type=f32)
            bc = bcol_v[pl.ds(r, TD), :]
            g = g + jnp.concatenate([bc] * (FH // 128), axis=1)
            u = (z1_v[pl.ds(r, TD), :].astype(f32) * g).astype(bf16)
            y2 = jnp.dot(u, wout_v[...], preferred_element_type=f32)
            out_v[pl.ds(r, TD), :] = (x1_v[pl.ds(r, TD), :] + mod_v[0:1, 5 * D:6 * D] * y2).astype(bf16)
        else:
            out_v[pl.ds(r, TD), :] = x_v[pl.ds(r, TD), :]
        if nd == 1:
            out_copy(i).start()
        else:
            @pl.when(ii >= (nd - 1) * (S // TD))
            def _():
                out_copy(i).start()
        return carry
    lax.fori_loop(0, nd * (S // TD), phase_d, 0)
    for i in range(S // TD):
        out_copy(i).wait()


def make(phases="ABCD"):
    @jax.jit
    def fn(A_x, A_wqkv, A_wo, B_x, B_w_in, B_w_sp, B_b_sp, B_w_out, c, w_mod):
        x = A_x.reshape(S, D)
        bsp = B_b_sp.reshape(1, S)
        any_spec = pl.BlockSpec(memory_space=pl.ANY)
        out = pl.pallas_call(
            functools.partial(_kernel, phases=phases),
            out_shape=jax.ShapeDtypeStruct((S, D), bf16),
            in_specs=[any_spec] * 9,
            out_specs=any_spec,
            scratch_shapes=[
                pltpu.VMEM((S, D), bf16),
                pltpu.VMEM((D, 3 * D), bf16),
                pltpu.VMEM((D, D), bf16),
                pltpu.VMEM((D, F), bf16),
                pltpu.VMEM((S, S), bf16),
                pltpu.VMEM((FH, D), bf16),
                pltpu.VMEM((D, 6 * D), bf16),
                pltpu.VMEM((D, D), bf16),
                pltpu.VMEM((D, D), bf16),
                pltpu.VMEM((S // 2, D), u32),
                pltpu.VMEM((SV, D), f32),
                pltpu.VMEM((H, DH, S), bf16),
                pltpu.VMEM((H, DH, S), f32),
                pltpu.VMEM((H, DH, S), bf16),
                pltpu.VMEM((D, S), bf16),
                pltpu.VMEM((DH, SV, 128), f32),
                pltpu.VMEM((DH, SV, 128), f32),
                pltpu.VMEM((S // 2, 128), u32),
                pltpu.VMEM((S // 2, 128), u32),
                pltpu.VMEM((NQ, S // 2, TQ), u32),
                pltpu.VMEM((NQ, S // 2, TQ), u32),
                pltpu.VMEM((8, S), f32),
                pltpu.VMEM((8, S), f32),
                pltpu.VMEM((8, TQ), f32),
                pltpu.VMEM((S, TF), f32),
                pltpu.VMEM((S, D), f32),
                pltpu.VMEM((S, FH), bf16),
                pltpu.VMEM((S, FH), bf16),
                pltpu.VMEM((S, 128), f32),
                pltpu.VMEM((8, 6 * D), f32),
                pltpu.VMEM((S, D), bf16),
                pltpu.VMEM((1, S), bf16),
                pltpu.VMEM((1, D), bf16),
                pltpu.VMEM((1, D), bf16),
                pltpu.SemaphoreType.DMA((10,)),
                pltpu.SemaphoreType.DMA((S // TD,)),
            ],
            compiler_params=pltpu.CompilerParams(vmem_limit_bytes=110 * 2 ** 20),
        )(x, A_wqkv, A_wo, B_w_in, B_w_sp, bsp, B_w_out, c, w_mod)
        return out.reshape(1, S, D)
    return fn


pallas_adaLN_cond__softmax_full_mha__mixer_gmlp__prompt_kernel = make()
```

```python
import math

import jax
import jax.numpy as jnp
from jax import lax
import jax.experimental.pallas as pl
import jax.experimental.pallas.tpu as pltpu

S = 2048
D = 512
H = 32
DH = 16
F = 1792
FH = 896
EPS = 1e-5
bf16 = jnp.bfloat16
f32 = jnp.float32
u32 = jnp.uint32

TQ = 128
NQ = S // TQ
SEG_M = 96
SEG_V = 16
NSEG = S // (SEG_M + SEG_V)
SEGS = [(i * (SEG_M + SEG_V), SEG_M, SEG_V) for i in range(NSEG)]
SEGS.append((NSEG * (SEG_M + SEG_V), S - NSEG * (SEG_M + SEG_V), 0))
SV = SEG_V * NSEG
PVK = 256
PVOFF = 192
NCH = 2
NL = 5
NPRE = 10
TK = 128
TF = 256
TA = 256
TA2 = 512
TC = 256
TD = 256
NA = S // TA
QSCALE = (DH ** -0.5) * math.log2(math.e)
L_LO = 2.0 ** -80
L_HI = 2.0 ** 100
V_MAX = 2.0 ** 20
NT = (((1,), (1,)), ((), ()))
TN = (((0,), (0,)), ((), ()))


def _ln(x):
    m = jnp.mean(x, axis=-1, keepdims=True)
    xc = x - m
    v = jnp.mean(xc * xc, axis=-1, keepdims=True)
    return xc * lax.rsqrt(v + EPS)


def _gelu(x):
    c = math.sqrt(2.0 / math.pi)
    return 0.5 * x * (1.0 + jnp.tanh(c * (x + 0.044715 * (x * x * x))))


def _p_store(p_ref, u, pair, ua, ub):
    r = u * (S // 4) + pair * 8
    if not isinstance(r, int):
        r = pl.multiple_of(r, 8)
    both = jnp.concatenate([ua, ub], axis=1).astype(bf16)
    p_ref[pl.ds(r, 8), :] = pltpu.bitcast(both, u32)


def _p_load(p_ref, u, k0, n):
    r = u * (S // 4) + k0 // 4
    if not isinstance(r, int):
        r = pl.multiple_of(r, 8)
    w = p_ref[pl.ds(r, n // 4), :]
    parts = []
    for t in range(n // 32):
        parts.append(w[t * 8:(t + 1) * 8, 0:TQ])
        parts.append(w[t * 8:(t + 1) * 8, TQ:2 * TQ])
    return pltpu.bitcast(jnp.concatenate(parts, axis=0), bf16)


def _kernel(x_hbm, wqkv_hbm, wo_hbm, win_hbm, wsp_hbm, bsp_hbm, wout_hbm, c_hbm, wmod_hbm,
            out_hbm,
            x_v, wqkv_v, wo_v, win_v, wsp_v, wout_v, wmod_v,
            wqT_v, wvT_v, h_v, k_v, kf_v, qT_v, qf_v, vT_v, oT_v,
            kb0, kb1, kr0, kr1, p0, p1, l0, l1, bad_v, sf_v,
            x1_v, z1_v, z2_v, bcol_v, mod_v, out_v, bsp_v, c_v,
            sems, xsems, osems):
    copies = {
        "c": (c_hbm, c_v),
        "wmod0": (wmod_hbm.at[:, 0:2 * D], wmod_v.at[:, 0:2 * D]),
        "wk": (wqkv_hbm.at[:, D:2 * D], wqkv_v.at[:, D:2 * D]),
        "wq": (wqkv_hbm.at[:, 0:D], wqkv_v.at[:, 0:D]),
        "wv": (wqkv_hbm.at[:, 2 * D:3 * D], wqkv_v.at[:, 2 * D:3 * D]),
        "wmod1": (wmod_hbm.at[:, 2 * D:6 * D], wmod_v.at[:, 2 * D:6 * D]),
        "bsp": (bsp_hbm, bsp_v),
        "wo": (wo_hbm, wo_v),
        "win": (win_hbm, win_v),
        "wout": (wout_hbm, wout_v),
        "wsp": (wsp_hbm, wsp_v),
    }
    cp = {name: pltpu.make_async_copy(src, dst, sems.at[i])
          for i, (name, (src, dst)) in enumerate(copies.items())}

    def x_copy(i):
        r = pl.multiple_of(i * TA, TA)
        return pltpu.make_async_copy(x_hbm.at[pl.ds(r, TA), :], x_v.at[pl.ds(r, TA), :], xsems.at[i])

    cp["c"].start()
    x_copy(0).start()
    cp["wmod0"].start()

    cp["c"].wait()
    cf = c_v[...].astype(f32)
    sc8 = jnp.broadcast_to((cf * jax.nn.sigmoid(cf)).astype(bf16), (8, D))
    x_copy(0).wait()
    cp["wk"].start()
    n0 = _ln(x_v[0:TA, :].astype(f32))
    cp["wmod0"].wait()
    x_copy(1).start()
    x_copy(2).start()
    mod_v[:, 0:2 * D] = jnp.dot(sc8, wmod_v[:, 0:2 * D], preferred_element_type=f32)

    def a_ln(i, n=None):
        r = pl.multiple_of(i * TA, TA)
        if n is None:
            n = _ln(x_v[pl.ds(r, TA), :].astype(f32))
        h = (n * (1.0 + mod_v[0:1, D:2 * D]) + mod_v[0:1, 0:D]).astype(bf16)
        h_v[pl.ds(r, TA), :] = h
        return h

    def a_k(i, h):
        kk = jnp.dot(h, wqkv_v[:, D:2 * D], preferred_element_type=f32)
        k_v[pl.ds(pl.multiple_of(i * (TA // 2), TA // 2), TA // 2), :] = pltpu.bitcast(kk.astype(bf16), u32)
        kf_v[pl.ds(pl.multiple_of(i * TA, TA), TA), :] = kk

    h0 = a_ln(0, n0)
    cp["wk"].wait()

    def phase_a1(i, h):
        @pl.when(i + 3 < NA)
        def _():
            x_copy(i + 3).start()

        @pl.when(i == 3)
        def _():
            cp["wq"].start()
            cp["wv"].start()
        x_copy(i + 1).wait()
        hn = a_ln(i + 1)
        a_k(i, h)
        return hn
    hl = lax.fori_loop(0, NA - 1, phase_a1, h0)
    cp["wq"].wait()
    cp["wv"].wait()
    for name in ("wmod1", "bsp", "wo", "win", "wout", "wsp"):
        cp[name].start()
    a_k(NA - 1, hl)
    wqT_v[...] = wqkv_v[:, 0:D].T
    wvT_v[...] = wqkv_v[:, 2 * D:3 * D].T

    def phase_a2(i, vm):
        r = pl.multiple_of(i * TA2, TA2)
        ht = h_v[pl.ds(r, TA2), :]
        qT = lax.dot_general(wqT_v[...], ht, NT, preferred_element_type=f32) * QSCALE
        qf_v[:, :, pl.ds(r, TA2)] = qT.reshape(H, DH, TA2)
        qT_v[:, :, pl.ds(r, TA2)] = qT.astype(bf16).reshape(H, DH, TA2)
        vT = lax.dot_general(wvT_v[...], ht, NT, preferred_element_type=f32)
        vT_v[:, :, pl.ds(r, TA2)] = vT.astype(bf16).reshape(H, DH, TA2)
        va = jnp.abs(vT).reshape(D // 8, 8, TA2).max(axis=0)
        for j in range(TA2 // 128):
            vm = jnp.maximum(vm, va[:, j * 128:(j + 1) * 128])
        return vm
    vmax = lax.fori_loop(0, S // TA2, phase_a2, jnp.zeros((8, 128), f32), unroll=2)
    bad_v[...] = jnp.where(vmax <= V_MAX, 0.0, 1.0)

    def build_k(h, kb, kr, do_kb=True):
        gl = pl.multiple_of((h // 8) * 128, 128)
        sh = (128 - (h % 8) * DH) % 128
        kr[...] = pltpu.roll(k_v[:, pl.ds(gl, 128)], sh, 1)
        if do_kb:
            kk = jnp.concatenate([kf_v[st + m:st + m + v, pl.ds(gl, 128)] for (st, m, v) in SEGS if v], axis=0)
            kk = pltpu.roll(kk, sh, 1)
            for d in range(DH):
                kb[d] = jnp.broadcast_to(kk[:, d:d + 1], (SV, 128))

    def block(u, hp, hc, p_rd, p_wr, l_rd, l_wr, kb_rd, kr_rd, use_vpu, bad):
        consume = hc is not None
        q0 = u * TQ
        qw = qT_v[hp, :, q0:q0 + TQ]
        l = [None] * NL
        acc = None
        npv = 0
        units = {}

        def put(n, val):
            units[n] = val
            if n ^ 1 in units:
                _p_store(p_wr, u, n // 2, units.pop(n & ~1), units.pop(n | 1))

        for i, (st, m, v) in enumerate(SEGS):
            parts = []
            if use_vpu and v:
                c0 = [None] * NCH
                c1 = [None] * NCH
                for d in range(DH):
                    qb = jnp.broadcast_to(qf_v[hp, d:d + 1, q0:q0 + TQ], (8, TQ))
                    t0 = kb_rd[d, i * SEG_V:i * SEG_V + 8, :] * qb
                    t1 = kb_rd[d, i * SEG_V + 8:i * SEG_V + 16, :] * qb
                    c0[d % NCH] = t0 if c0[d % NCH] is None else c0[d % NCH] + t0
                    c1[d % NCH] = t1 if c1[d % NCH] is None else c1[d % NCH] + t1
                e0 = jnp.exp2(sum(c0[1:], c0[0]))
                e1 = jnp.exp2(sum(c1[1:], c1[0]))
                parts.append(e0 + e1)
                put((st + m) // 16, jnp.concatenate([e0, e1], axis=0))
            sz = m if use_vpu else m + v
            kk = pltpu.bitcast(kr_rd[st // 2:(st + sz) // 2, :], bf16)[:, 0:DH]
            p = jnp.exp2(jnp.dot(kk, qw, preferred_element_type=f32))
            for r in range(sz // 16):
                parts.append(p[r * 16:r * 16 + 8] + p[r * 16 + 8:r * 16 + 16])
            for t in parts:
                l[i % NL] = t if l[i % NL] is None else l[i % NL] + t
            for r in range(sz // 16):
                put(st // 16 + r, p[r * 16:(r + 1) * 16])
            while consume and npv < S // PVK and (npv + 1) * PVK <= st + m + v + PVOFF:
                k0 = npv * PVK
                t = jnp.dot(vT_v[hc, :, k0:k0 + PVK], _p_load(p_rd, u, k0, PVK), preferred_element_type=f32)
                acc = t if acc is None else acc + t
                npv += 1
        if consume:
            ls = l_rd[:, q0:q0 + TQ].sum(axis=0, keepdims=True)
            oT_v[pl.ds(pl.multiple_of(hc * DH, DH), DH), q0:q0 + TQ] = (acc * (1.0 / ls)).astype(bf16)
            bad = jnp.where((ls >= L_LO) & (ls <= L_HI), bad, 1.0)
        l_wr[:, q0:q0 + TQ] = sum(l[1:], l[0])
        return bad

    def mod_rest(j):
        c0 = 2 * D + j * 128
        mod_v[:, c0:c0 + 128] = jnp.dot(sc8, wmod_v[:, c0:c0 + 128], preferred_element_type=f32)
        bj = jnp.broadcast_to(bsp_v[:, j * 128:(j + 1) * 128].astype(f32), (128, 128))
        bcol_v[j * 128:(j + 1) * 128, :] = bj.T

    def step(h, p_rd, p_wr, l_rd, l_wr, kb_rd, kr_rd, kb_wr, kr_wr, first=False):
        bad = None if first else bad_v[...]
        for u in range(NQ):
            if first:
                mod_rest(u)
            bad = block(u, h + 1, None if first else h, p_rd, p_wr, l_rd, l_wr, kb_rd, kr_rd, not first, bad)
        if not first:
            bad_v[...] = bad
        build_k(jnp.minimum(h + 2, H - 1), kb_wr, kr_wr)

    cp["wmod1"].wait()
    cp["bsp"].wait()
    build_k(0, kb0, kr0, do_kb=False)
    step(-1, None, p0, None, l0, kb0, kr0, kb1, kr1, first=True)

    def phase_b(h, carry):
        lax.cond(h % 2 == 0,
                 lambda: step(h, p0, p1, l0, l1, kb1, kr1, kb0, kr0),
                 lambda: step(h, p1, p0, l1, l0, kb0, kr0, kb1, kr1))
        return carry
    lax.fori_loop(0, H - 1, phase_b, 0)
    lsl = l1[...].sum(axis=0, keepdims=True)
    badl = jnp.where((lsl >= L_LO) & (lsl <= L_HI), 0.0, 1.0)
    bad = bad_v[...]
    for j in range(NQ):
        bad = jnp.maximum(bad, badl[:, j * TQ:(j + 1) * TQ])

    @pl.when(jnp.max(bad) > 0.0)
    def _():
        row = lax.broadcasted_iota(jnp.int32, (128, TF), 0) // DH

        def exact(b, carry):
            h = b // (S // TF)
            q0 = pl.multiple_of((b % (S // TF)) * TF, TF)
            ub = (b % (S // TF)) * (TF // TQ)
            g = h // 8
            gl = pl.multiple_of(g * 128, 128)
            qg = qf_v[pl.ds(g * 8, 8), :, pl.ds(q0, TF)].reshape(128, TF)
            qw = jnp.where(row == h % 8, qg, 0.0).astype(bf16)
            mx = jnp.full((8, TF), -jnp.inf, f32)
            for c in range(S // TK):
                kk = pltpu.bitcast(k_v[c * TK // 2:(c + 1) * TK // 2, pl.ds(gl, 128)], bf16)
                s = jnp.dot(kk, qw, preferred_element_type=f32)
                sf_v[c * TK:(c + 1) * TK, :] = s
                mx = jnp.maximum(mx, s.reshape(TK // 8, 8, TF).max(axis=0))
            m = mx.max(axis=0, keepdims=True)
            l = jnp.zeros((8, TF), f32)
            acc = jnp.zeros((DH, TF), f32)
            for c in range(S // TK):
                p = jnp.exp2(sf_v[c * TK:(c + 1) * TK, :] - m)
                l = l + p.reshape(TK // 8, 8, TF).sum(axis=0)
                for j in range(TF // TQ):
                    for t in range(TK // 32):
                        _p_store(p1, ub + j, c * (TK // 32) + t, p[t * 32:t * 32 + 16, j * TQ:(j + 1) * TQ],
                                 p[t * 32 + 16:t * 32 + 32, j * TQ:(j + 1) * TQ])
                acc = acc + jnp.dot(vT_v[h, :, c * TK:(c + 1) * TK], p.astype(bf16),
                                    preferred_element_type=f32)
            l1[:, pl.ds(q0, TF)] = l
            o = acc / l.sum(axis=0, keepdims=True)
            oT_v[pl.ds(pl.multiple_of(h * DH, DH), DH), pl.ds(q0, TF)] = o.astype(bf16)
            return carry
        lax.fori_loop(0, H * (S // TF), exact, 0)

    cp["wo"].wait()
    cp["win"].wait()

    def c_s1(i):
        r = pl.multiple_of(i * TC, TC)
        y = lax.dot_general(oT_v[:, pl.ds(r, TC)], wo_v[...], TN, preferred_element_type=f32)
        x1 = x_v[pl.ds(r, TC), :].astype(f32) + mod_v[0:1, 2 * D:3 * D] * y
        x1_v[pl.ds(r, TC), :] = x1
        return (_ln(x1) * (1.0 + mod_v[0:1, 4 * D:5 * D]) + mod_v[0:1, 3 * D:4 * D]).astype(bf16)

    def c_z2(i, h2):
        r = pl.multiple_of(i * TC, TC)
        z2 = _gelu(jnp.dot(h2, win_v[:, FH:F], preferred_element_type=f32))
        z2_v[pl.ds(r, TC), :] = _ln(z2).astype(bf16)

    def c_z1(i, h2):
        r = pl.multiple_of(i * TC, TC)
        z1_v[pl.ds(r, TC), :] = jnp.dot(h2, win_v[:, 0:FH], preferred_element_type=f32).astype(bf16)

    def last_pv(u):
        q0 = u * TQ if isinstance(u, int) else pl.multiple_of(u * TQ, TQ)
        acc = None
        for c in range(S // PVK):
            k0 = c * PVK
            t = jnp.dot(vT_v[H - 1, :, k0:k0 + PVK], _p_load(p1, u, k0, PVK), preferred_element_type=f32)
            acc = t if acc is None else acc + t
        ls = l1[:, pl.ds(q0, TQ)].sum(axis=0, keepdims=True)
        oT_v[(H - 1) * DH:H * DH, pl.ds(q0, TQ)] = (acc * (1.0 / ls)).astype(bf16)

    last_pv(0)
    last_pv(1)
    h20 = c_s1(0)
    for u in range(2, NPRE):
        last_pv(u)

    def phase_c(i, h2):
        c_z2(i, h2)
        hn = c_s1(i + 1)
        last_pv(jnp.minimum(NPRE + i, NQ - 1))
        c_z1(i, h2)
        return hn
    h2 = lax.fori_loop(0, S // TC - 1, phase_c, h20)
    c_z2(S // TC - 1, h2)
    c_z1(S // TC - 1, h2)

    cp["wsp"].wait()
    cp["wout"].wait()

    def out_copy(i):
        r = pl.multiple_of(i * TD, TD)
        return pltpu.make_async_copy(out_v.at[pl.ds(r, TD), :], out_hbm.at[pl.ds(r, TD), :], osems.at[i])

    def phase_d(i, carry):
        r = pl.multiple_of(i * TD, TD)
        g = jnp.dot(wsp_v[pl.ds(r, TD), :], z2_v[...], preferred_element_type=f32)
        g = g + jnp.concatenate([bcol_v[pl.ds(r, TD), :]] * (FH // 128), axis=1)
        u = (_gelu(z1_v[pl.ds(r, TD), :].astype(f32)) * g).astype(bf16)
        y2 = jnp.dot(u, wout_v[...], preferred_element_type=f32)
        out_v[pl.ds(r, TD), :] = (x1_v[pl.ds(r, TD), :] + mod_v[0:1, 5 * D:6 * D] * y2).astype(bf16)
        out_copy(i).start()
        return carry
    lax.fori_loop(0, S // TD, phase_d, 0, unroll=2)
    for i in range(S // TD):
        out_copy(i).wait()


@jax.jit
def pallas_adaLN_cond__softmax_full_mha__mixer_gmlp__prompt_kernel(
    A_x: jax.Array,
    A_wqkv: jax.Array,
    A_wo: jax.Array,
    B_x: jax.Array,
    B_w_in: jax.Array,
    B_w_sp: jax.Array,
    B_b_sp: jax.Array,
    B_w_out: jax.Array,
    c: jax.Array,
    w_mod: jax.Array,
):
    del B_x
    any_spec = pl.BlockSpec(memory_space=pl.ANY)
    out = pl.pallas_call(
        _kernel,
        out_shape=jax.ShapeDtypeStruct((S, D), bf16),
        in_specs=[any_spec] * 9,
        out_specs=any_spec,
        scratch_shapes=[
            pltpu.VMEM((S, D), bf16),
            pltpu.VMEM((D, 3 * D), bf16),
            pltpu.VMEM((D, D), bf16),
            pltpu.VMEM((D, F), bf16),
            pltpu.VMEM((S, S), bf16),
            pltpu.VMEM((FH, D), bf16),
            pltpu.VMEM((D, 6 * D), bf16),
            pltpu.VMEM((D, D), bf16),
            pltpu.VMEM((D, D), bf16),
            pltpu.VMEM((S, D), bf16),
            pltpu.VMEM((S // 2, D), u32),
            pltpu.VMEM((S, D), f32),
            pltpu.VMEM((H, DH, S), bf16),
            pltpu.VMEM((H, DH, S), f32),
            pltpu.VMEM((H, DH, S), bf16),
            pltpu.VMEM((D, S), bf16),
            pltpu.VMEM((DH, SV, 128), f32),
            pltpu.VMEM((DH, SV, 128), f32),
            pltpu.VMEM((S // 2, 128), u32),
            pltpu.VMEM((S // 2, 128), u32),
            pltpu.VMEM((NQ * S // 4, 2 * TQ), u32),
            pltpu.VMEM((NQ * S // 4, 2 * TQ), u32),
            pltpu.VMEM((8, S), f32),
            pltpu.VMEM((8, S), f32),
            pltpu.VMEM((8, TQ), f32),
            pltpu.VMEM((S, TF), f32),
            pltpu.VMEM((S, D), f32),
            pltpu.VMEM((S, FH), bf16),
            pltpu.VMEM((S, FH), bf16),
            pltpu.VMEM((S, 128), f32),
            pltpu.VMEM((8, 6 * D), f32),
            pltpu.VMEM((S, D), bf16),
            pltpu.VMEM((1, S), bf16),
            pltpu.VMEM((1, D), bf16),
            pltpu.SemaphoreType.DMA((11,)),
            pltpu.SemaphoreType.DMA((NA,)),
            pltpu.SemaphoreType.DMA((S // TD,)),
        ],
        compiler_params=pltpu.CompilerParams(vmem_limit_bytes=110 * 2 ** 20),
    )(A_x.reshape(S, D), A_wqkv, A_wo, B_w_in, B_w_sp, B_b_sp.reshape(1, S), B_w_out, c, w_mod)
    return out.reshape(1, S, D)
```

```python
import math

import jax
import jax.numpy as jnp
from jax import lax
import jax.experimental.pallas as pl
import jax.experimental.pallas.tpu as pltpu

S = 2048
D = 512
H = 32
DH = 16
F = 1792
FH = 896
EPS = 1e-5
bf16 = jnp.bfloat16
f32 = jnp.float32
u32 = jnp.uint32

TQ = 128
NQ = S // TQ
SEG_V = 16
_PAT = [(48, 48), (48, 32), (48, 32)]
SEGS = []
_st = 0
while _st < S:
    _ma, _mb = _PAT[len(SEGS) % len(_PAT)]
    if _st + _ma + _mb + SEG_V > S:
        SEGS.append((_st, S - _st, 0, 0))
        _st = S
    else:
        SEGS.append((_st, _ma, _mb, SEG_V))
        _st += _ma + _mb + SEG_V
SV = sum(seg[3] for seg in SEGS)
PVK = 128
NCH = 2
NL = 3
NPRE = 10
TK = 128
TF = 256
TA = 256
TA2 = 512
TC = 256
TD = 256
NA = S // TA
QSCALE = (DH ** -0.5) * math.log2(math.e)
L_LO = 2.0 ** -80
L_HI = 2.0 ** 100
V_MAX = 2.0 ** 20
NT = (((1,), (1,)), ((), ()))
TN = (((0,), (0,)), ((), ()))


def _ln(x):
    m = jnp.mean(x, axis=-1, keepdims=True)
    xc = x - m
    v = jnp.mean(xc * xc, axis=-1, keepdims=True)
    return xc * lax.rsqrt(v + EPS)


def _gelu(x):
    c = math.sqrt(2.0 / math.pi)
    return 0.5 * x * (1.0 + jnp.tanh(c * (x + 0.044715 * (x * x * x))))


def _p_store(p_ref, u, pair, ua, ub):
    r = u * (S // 4) + pair * 8
    if not isinstance(r, int):
        r = pl.multiple_of(r, 8)
    both = jnp.concatenate([ua, ub], axis=1).astype(bf16)
    p_ref[pl.ds(r, 8), :] = pltpu.bitcast(both, u32)


def _p_load(p_ref, u, k0, n):
    r = u * (S // 4) + k0 // 4
    if not isinstance(r, int):
        r = pl.multiple_of(r, 8)
    w = p_ref[pl.ds(r, n // 4), :]
    parts = []
    for t in range(n // 32):
        parts.append(w[t * 8:(t + 1) * 8, 0:TQ])
        parts.append(w[t * 8:(t + 1) * 8, TQ:2 * TQ])
    return pltpu.bitcast(jnp.concatenate(parts, axis=0), bf16)


def _head(ref, h, c0, n):
    r = h * (DH // 2)
    if not isinstance(r, int):
        r = pl.multiple_of(r, DH // 2)
    return pltpu.bitcast(ref[pl.ds(r, DH // 2), c0:c0 + n], bf16)


def _kernel(x_hbm, wqkv_hbm, wo_hbm, win_hbm, wsp_hbm, bsp_hbm, wout_hbm, c_hbm, wmod_hbm,
            out_hbm,
            x_v, wqkv_v, wo_v, win_v, wsp_v, wout_v, wmod_v,
            wqT_v, wvT_v, h_v, k_v, kf_v, qT_v, qf_v, vT_v, oT_v,
            kb0, kb1, kr0, kr1, p0, p1, l0, l1, bad_v, sf_v,
            x1_v, z1_v, z2_v, bcol_v, mod_v, out_v, bsp_v, c_v,
            sems, xsems, osems):
    copies = {
        "c": (c_hbm, c_v),
        "wmod0": (wmod_hbm.at[:, 0:2 * D], wmod_v.at[:, 0:2 * D]),
        "wk": (wqkv_hbm.at[:, D:2 * D], wqkv_v.at[:, D:2 * D]),
        "wq": (wqkv_hbm.at[:, 0:D], wqkv_v.at[:, 0:D]),
        "wv": (wqkv_hbm.at[:, 2 * D:3 * D], wqkv_v.at[:, 2 * D:3 * D]),
        "wmod1": (wmod_hbm.at[:, 2 * D:6 * D], wmod_v.at[:, 2 * D:6 * D]),
        "bsp": (bsp_hbm, bsp_v),
        "wo": (wo_hbm, wo_v),
        "win": (win_hbm, win_v),
        "wout": (wout_hbm, wout_v),
        "wsp": (wsp_hbm, wsp_v),
    }
    cp = {name: pltpu.make_async_copy(src, dst, sems.at[i])
          for i, (name, (src, dst)) in enumerate(copies.items())}

    def x_copy(i):
        r = pl.multiple_of(i * TA, TA)
        return pltpu.make_async_copy(x_hbm.at[pl.ds(r, TA), :], x_v.at[pl.ds(r, TA), :], xsems.at[i])

    cp["c"].start()
    x_copy(0).start()
    cp["wmod0"].start()

    cp["c"].wait()
    cf = c_v[...].astype(f32)
    sc8 = jnp.broadcast_to((cf * jax.nn.sigmoid(cf)).astype(bf16), (8, D))
    x_copy(0).wait()
    cp["wk"].start()
    n0 = _ln(x_v[0:TA, :].astype(f32))
    cp["wmod0"].wait()
    x_copy(1).start()
    x_copy(2).start()
    mod_v[:, 0:2 * D] = jnp.dot(sc8, wmod_v[:, 0:2 * D], preferred_element_type=f32)

    def a_ln(i, n=None):
        r = pl.multiple_of(i * TA, TA)
        if n is None:
            n = _ln(x_v[pl.ds(r, TA), :].astype(f32))
        h = (n * (1.0 + mod_v[0:1, D:2 * D]) + mod_v[0:1, 0:D]).astype(bf16)
        h_v[pl.ds(r, TA), :] = h
        return h

    def a_k(i, h):
        kk = jnp.dot(h, wqkv_v[:, D:2 * D], preferred_element_type=f32)
        k_v[pl.ds(pl.multiple_of(i * (TA // 2), TA // 2), TA // 2), :] = pltpu.bitcast(kk.astype(bf16), u32)
        kf_v[pl.ds(pl.multiple_of(i * TA, TA), TA), :] = kk

    h0 = a_ln(0, n0)
    cp["wk"].wait()

    def phase_a1(i, h):
        @pl.when(i + 3 < NA)
        def _():
            x_copy(i + 3).start()

        @pl.when(i == 3)
        def _():
            cp["wq"].start()
            cp["wv"].start()
        x_copy(i + 1).wait()
        hn = a_ln(i + 1)
        a_k(i, h)
        return hn
    hl = lax.fori_loop(0, NA - 1, phase_a1, h0)
    cp["wq"].wait()
    cp["wv"].wait()
    for name in ("wmod1", "bsp", "wo", "win", "wout", "wsp"):
        cp[name].start()
    a_k(NA - 1, hl)
    wqT_v[...] = wqkv_v[:, 0:D].T
    wvT_v[...] = wqkv_v[:, 2 * D:3 * D].T

    def phase_a2(i, vm):
        r = pl.multiple_of(i * TA2, TA2)
        ht = h_v[pl.ds(r, TA2), :]
        qT = lax.dot_general(wqT_v[...], ht, NT, preferred_element_type=f32) * QSCALE
        qf_v[:, :, pl.ds(r, TA2)] = qT.reshape(H, DH, TA2)
        qT_v[:, pl.ds(r, TA2)] = pltpu.bitcast(qT.astype(bf16), u32)
        vT = lax.dot_general(wvT_v[...], ht, NT, preferred_element_type=f32)
        vT_v[:, pl.ds(r, TA2)] = pltpu.bitcast(vT.astype(bf16), u32)
        va = jnp.abs(vT).reshape(D // 8, 8, TA2).max(axis=0)
        for j in range(TA2 // 128):
            vm = jnp.maximum(vm, va[:, j * 128:(j + 1) * 128])
        return vm
    vmax = lax.fori_loop(0, S // TA2, phase_a2, jnp.zeros((8, 128), f32), unroll=2)
    bad_v[...] = jnp.where(vmax <= V_MAX, 0.0, 1.0)

    def build_k(h, kb, kr, do_kb=True):
        gl = pl.multiple_of((h // 8) * 128, 128)
        sh = (128 - (h % 8) * DH) % 128
        kr[...] = pltpu.roll(k_v[:, pl.ds(gl, 128)], sh, 1)
        if do_kb:
            kk = jnp.concatenate([kf_v[st + ma + mb:st + ma + mb + v, pl.ds(gl, 128)]
                                  for (st, ma, mb, v) in SEGS if v], axis=0)
            kk = pltpu.roll(kk, sh, 1)
            for d in range(DH):
                kb[d] = jnp.broadcast_to(kk[:, d:d + 1], (SV, 128))

    def block(u, hp, hc, p_rd, p_wr, l_rd, l_wr, kb_rd, kr_rd, use_vpu, bad):
        consume = hc is not None
        q0 = u * TQ
        qw = _head(qT_v, hp, q0, TQ)
        l = [None] * NL
        acc = None
        npv = 0
        units = {}

        def ladd(li, t):
            l[li] = t if l[li] is None else l[li] + t

        def put(n, val):
            units[n] = val
            if n ^ 1 in units:
                _p_store(p_wr, u, n // 2, units.pop(n & ~1), units.pop(n | 1))

        def vpu8(o):
            cc = [None] * NCH
            for d in range(DH):
                t = kb_rd[d, o:o + 8, :] * jnp.broadcast_to(qf_v[hp, d:d + 1, q0:q0 + TQ], (8, TQ))
                cc[d % NCH] = t if cc[d % NCH] is None else cc[d % NCH] + t
            return jnp.exp2(sum(cc[1:], cc[0]))

        def qk(a, b, li):
            kk = pltpu.bitcast(kr_rd[a // 2:b // 2, :], bf16)[:, 0:DH]
            p = jnp.exp2(jnp.dot(kk, qw, preferred_element_type=f32))
            for r in range((b - a) // 16):
                ladd(li, p[r * 16:r * 16 + 8] + p[r * 16 + 8:r * 16 + 16])
            for r in range((b - a) // 16):
                put(a // 16 + r, p[r * 16:(r + 1) * 16])

        for i, (st, ma, mb, v) in enumerate(SEGS):
            end = st + ma + mb + v
            if use_vpu and v:
                la = (2 * i) % NL
                lb = (2 * i + 1) % NL
                e0 = vpu8(i * SEG_V)
                ladd(la, e0)
                qk(st, st + ma, la)
                e1 = vpu8(i * SEG_V + 8)
                ladd(lb, e1)
                put((end - v) // 16, jnp.concatenate([e0, e1], axis=0))
                qk(st + ma, st + ma + mb, lb)
            else:
                qk(st, end, (2 * i) % NL)
            while consume and (npv + 1) * PVK <= end:
                k0 = npv * PVK
                t = jnp.dot(_head(vT_v, hc, k0, PVK), _p_load(p_rd, u, k0, PVK), preferred_element_type=f32)
                acc = t if acc is None else acc + t
                npv += 1
        if consume:
            ls = l_rd[:, q0:q0 + TQ].sum(axis=0, keepdims=True)
            oT_v[pl.ds(pl.multiple_of(hc * DH, DH), DH), q0:q0 + TQ] = (acc * (1.0 / ls)).astype(bf16)
            bad = jnp.where((ls >= L_LO) & (ls <= L_HI), bad, 1.0)
        l_wr[:, q0:q0 + TQ] = sum(l[1:], l[0])
        return bad

    def mod_rest(j):
        c0 = 2 * D + j * 128
        mod_v[:, c0:c0 + 128] = jnp.dot(sc8, wmod_v[:, c0:c0 + 128], preferred_element_type=f32)
        bj = jnp.broadcast_to(bsp_v[...].astype(f32).reshape(1, S)[:, j * 128:(j + 1) * 128], (128, 128))
        bcol_v[j * 128:(j + 1) * 128, :] = bj.T

    def step(h, p_rd, p_wr, l_rd, l_wr, kb_rd, kr_rd, kb_wr, kr_wr, first=False):
        bad = None if first else bad_v[...]
        for u in range(NQ):
            if first:
                mod_rest(u)
            bad = block(u, h + 1, None if first else h, p_rd, p_wr, l_rd, l_wr, kb_rd, kr_rd, not first, bad)
        if not first:
            bad_v[...] = bad
        build_k(jnp.minimum(h + 2, H - 1), kb_wr, kr_wr)

    cp["wmod1"].wait()
    cp["bsp"].wait()
    build_k(0, kb0, kr0, do_kb=False)
    step(-1, None, p0, None, l0, kb0, kr0, kb1, kr1, first=True)

    def phase_b(h, carry):
        lax.cond(h % 2 == 0,
                 lambda: step(h, p0, p1, l0, l1, kb1, kr1, kb0, kr0),
                 lambda: step(h, p1, p0, l1, l0, kb0, kr0, kb1, kr1))
        return carry
    lax.fori_loop(0, H - 1, phase_b, 0)
    lsl = l1[...].sum(axis=0, keepdims=True)
    badl = jnp.where((lsl >= L_LO) & (lsl <= L_HI), 0.0, 1.0)
    bad = bad_v[...]
    for j in range(NQ):
        bad = jnp.maximum(bad, badl[:, j * TQ:(j + 1) * TQ])

    @pl.when(jnp.max(bad) > 0.0)
    def _():
        row = lax.broadcasted_iota(jnp.int32, (128, TF), 0) // DH

        def exact(b, carry):
            h = b // (S // TF)
            q0 = pl.multiple_of((b % (S // TF)) * TF, TF)
            ub = (b % (S // TF)) * (TF // TQ)
            g = h // 8
            gl = pl.multiple_of(g * 128, 128)
            qg = qf_v[pl.ds(g * 8, 8), :, pl.ds(q0, TF)].reshape(128, TF)
            qw = jnp.where(row == h % 8, qg, 0.0).astype(bf16)
            mx = jnp.full((8, TF), -jnp.inf, f32)
            for c in range(S // TK):
                kk = pltpu.bitcast(k_v[c * TK // 2:(c + 1) * TK // 2, pl.ds(gl, 128)], bf16)
                s = jnp.dot(kk, qw, preferred_element_type=f32)
                sf_v[c * TK:(c + 1) * TK, :] = s
                mx = jnp.maximum(mx, s.reshape(TK // 8, 8, TF).max(axis=0))
            m = mx.max(axis=0, keepdims=True)
            l = jnp.zeros((8, TF), f32)
            acc = jnp.zeros((DH, TF), f32)
            for c in range(S // TK):
                p = jnp.exp2(sf_v[c * TK:(c + 1) * TK, :] - m)
                l = l + p.reshape(TK // 8, 8, TF).sum(axis=0)
                for j in range(TF // TQ):
                    for t in range(TK // 32):
                        _p_store(p1, ub + j, c * (TK // 32) + t, p[t * 32:t * 32 + 16, j * TQ:(j + 1) * TQ],
                                 p[t * 32 + 16:t * 32 + 32, j * TQ:(j + 1) * TQ])
                acc = acc + jnp.dot(_head(vT_v, h, c * TK, TK), p.astype(bf16),
                                    preferred_element_type=f32)
            l1[:, pl.ds(q0, TF)] = l
            o = acc / l.sum(axis=0, keepdims=True)
            oT_v[pl.ds(pl.multiple_of(h * DH, DH), DH), pl.ds(q0, TF)] = o.astype(bf16)
            return carry
        lax.fori_loop(0, H * (S // TF), exact, 0)

    cp["wo"].wait()
    cp["win"].wait()

    def c_s1(i):
        r = pl.multiple_of(i * TC, TC)
        y = lax.dot_general(oT_v[:, pl.ds(r, TC)], wo_v[...], TN, preferred_element_type=f32)
        x1 = x_v[pl.ds(r, TC), :].astype(f32) + mod_v[0:1, 2 * D:3 * D] * y
        x1_v[pl.ds(r, TC), :] = x1
        return (_ln(x1) * (1.0 + mod_v[0:1, 4 * D:5 * D]) + mod_v[0:1, 3 * D:4 * D]).astype(bf16)

    def c_z2(i, h2):
        r = pl.multiple_of(i * TC, TC)
        z2 = _gelu(jnp.dot(h2, win_v[:, FH:F], preferred_element_type=f32))
        z2_v[pl.ds(r, TC), :] = _ln(z2).astype(bf16)

    def c_z1(i, h2):
        r = pl.multiple_of(i * TC, TC)
        z1_v[pl.ds(r, TC), :] = jnp.dot(h2, win_v[:, 0:FH], preferred_element_type=f32).astype(bf16)

    def last_pv(u):
        q0 = u * TQ if isinstance(u, int) else pl.multiple_of(u * TQ, TQ)
        acc = None
        for c in range(S // PVK):
            k0 = c * PVK
            t = jnp.dot(_head(vT_v, H - 1, k0, PVK), _p_load(p1, u, k0, PVK), preferred_element_type=f32)
            acc = t if acc is None else acc + t
        ls = l1[:, pl.ds(q0, TQ)].sum(axis=0, keepdims=True)
        oT_v[(H - 1) * DH:H * DH, pl.ds(q0, TQ)] = (acc * (1.0 / ls)).astype(bf16)

    last_pv(0)
    last_pv(1)
    h20 = c_s1(0)
    for u in range(2, NPRE):
        last_pv(u)

    def phase_c(i, h2):
        c_z2(i, h2)
        hn = c_s1(i + 1)
        c_z1(i, h2)
        last_pv(jnp.minimum(NPRE + i, NQ - 1))
        return hn
    h2 = lax.fori_loop(0, S // TC - 1, phase_c, h20)
    c_z2(S // TC - 1, h2)
    c_z1(S // TC - 1, h2)

    cp["wsp"].wait()
    cp["wout"].wait()

    def out_copy(i):
        r = pl.multiple_of(i * TD, TD)
        return pltpu.make_async_copy(out_v.at[pl.ds(r, TD), :], out_hbm.at[pl.ds(r, TD), :], osems.at[i])

    def phase_d(i, carry):
        r = pl.multiple_of(i * TD, TD)
        g = jnp.dot(wsp_v[pl.ds(r, TD), :], z2_v[...], preferred_element_type=f32)
        g = g + jnp.concatenate([bcol_v[pl.ds(r, TD), :]] * (FH // 128), axis=1)
        u = (_gelu(z1_v[pl.ds(r, TD), :].astype(f32)) * g).astype(bf16)
        y2 = jnp.dot(u, wout_v[...], preferred_element_type=f32)
        out_v[pl.ds(r, TD), :] = (x1_v[pl.ds(r, TD), :] + mod_v[0:1, 5 * D:6 * D] * y2).astype(bf16)
        out_copy(i).start()
        return carry
    lax.fori_loop(0, S // TD, phase_d, 0, unroll=2)
    for i in range(S // TD):
        out_copy(i).wait()


@jax.jit
def pallas_adaLN_cond__softmax_full_mha__mixer_gmlp__prompt_kernel(
    A_x: jax.Array,
    A_wqkv: jax.Array,
    A_wo: jax.Array,
    B_x: jax.Array,
    B_w_in: jax.Array,
    B_w_sp: jax.Array,
    B_b_sp: jax.Array,
    B_w_out: jax.Array,
    c: jax.Array,
    w_mod: jax.Array,
):
    del B_x
    any_spec = pl.BlockSpec(memory_space=pl.ANY)
    out = pl.pallas_call(
        _kernel,
        out_shape=jax.ShapeDtypeStruct((S, D), bf16),
        in_specs=[any_spec] * 9,
        out_specs=any_spec,
        scratch_shapes=[
            pltpu.VMEM((S, D), bf16),
            pltpu.VMEM((D, 3 * D), bf16),
            pltpu.VMEM((D, D), bf16),
            pltpu.VMEM((D, F), bf16),
            pltpu.VMEM((S, S), bf16),
            pltpu.VMEM((FH, D), bf16),
            pltpu.VMEM((D, 6 * D), bf16),
            pltpu.VMEM((D, D), bf16),
            pltpu.VMEM((D, D), bf16),
            pltpu.VMEM((S, D), bf16),
            pltpu.VMEM((S // 2, D), u32),
            pltpu.VMEM((S, D), f32),
            pltpu.VMEM((D // 2, S), u32),
            pltpu.VMEM((H, DH, S), f32),
            pltpu.VMEM((D // 2, S), u32),
            pltpu.VMEM((D, S), bf16),
            pltpu.VMEM((DH, SV, 128), f32),
            pltpu.VMEM((DH, SV, 128), f32),
            pltpu.VMEM((S // 2, 128), u32),
            pltpu.VMEM((S // 2, 128), u32),
            pltpu.VMEM((NQ * S // 4, 2 * TQ), u32),
            pltpu.VMEM((NQ * S // 4, 2 * TQ), u32),
            pltpu.VMEM((8, S), f32),
            pltpu.VMEM((8, S), f32),
            pltpu.VMEM((8, TQ), f32),
            pltpu.VMEM((S, TF), f32),
            pltpu.VMEM((S, D), f32),
            pltpu.VMEM((S, FH), bf16),
            pltpu.VMEM((S, FH), bf16),
            pltpu.VMEM((S, 128), f32),
            pltpu.VMEM((8, 6 * D), f32),
            pltpu.VMEM((S, D), bf16),
            pltpu.VMEM((S,), bf16),
            pltpu.VMEM((1, D), bf16),
            pltpu.SemaphoreType.DMA((11,)),
            pltpu.SemaphoreType.DMA((NA,)),
            pltpu.SemaphoreType.DMA((S // TD,)),
        ],
        compiler_params=pltpu.CompilerParams(vmem_limit_bytes=110 * 2 ** 20),
    )(A_x.reshape(S, D), A_wqkv, A_wo, B_w_in, B_w_sp, B_b_sp, B_w_out, c, w_mod)
    return out.reshape(1, S, D)
```

```python
import math

import jax
import jax.numpy as jnp
from jax import lax
import jax.experimental.pallas as pl
import jax.experimental.pallas.tpu as pltpu

S = 2048
D = 512
H = 32
DH = 16
F = 1792
FH = 896
EPS = 1e-5
bf16 = jnp.bfloat16
f32 = jnp.float32
u32 = jnp.uint32

TQ = 128
NQ = S // TQ
SEG_V = 16
_PAT = [(48, 48), (48, 32), (48, 32)]
SEGS = []
_st = 0
while _st < S:
    _ma, _mb = _PAT[len(SEGS) % len(_PAT)]
    if _st + _ma + _mb + SEG_V > S:
        SEGS.append((_st, S - _st, 0, 0))
        _st = S
    else:
        SEGS.append((_st, _ma, _mb, SEG_V))
        _st += _ma + _mb + SEG_V
SV = sum(seg[3] for seg in SEGS)
PVK = 128
NCH = 2
NL = 3
NPRE = 10
TK = 128
TF = 256
TA = 256
TA2 = 512
TC = 256
TD = 256
NA = S // TA
QSCALE = (DH ** -0.5) * math.log2(math.e)
L_LO = 2.0 ** -80
L_HI = 2.0 ** 100
V_MAX = 2.0 ** 20
NT = (((1,), (1,)), ((), ()))
TN = (((0,), (0,)), ((), ()))


def _ln(x):
    m = jnp.mean(x, axis=-1, keepdims=True)
    xc = x - m
    v = jnp.mean(xc * xc, axis=-1, keepdims=True)
    return xc * lax.rsqrt(v + EPS)


def _gelu(x):
    c = math.sqrt(2.0 / math.pi)
    return 0.5 * x * (1.0 + jnp.tanh(c * (x + 0.044715 * (x * x * x))))


def _p_store(p_ref, u, pair, ua, ub):
    r = u * (S // 4) + pair * 8
    if not isinstance(r, int):
        r = pl.multiple_of(r, 8)
    both = jnp.concatenate([ua, ub], axis=1).astype(bf16)
    p_ref[pl.ds(r, 8), :] = pltpu.bitcast(both, u32)


def _p_load(p_ref, u, k0, n):
    r = u * (S // 4) + k0 // 4
    if not isinstance(r, int):
        r = pl.multiple_of(r, 8)
    w = p_ref[pl.ds(r, n // 4), :]
    parts = []
    for t in range(n // 32):
        parts.append(w[t * 8:(t + 1) * 8, 0:TQ])
        parts.append(w[t * 8:(t + 1) * 8, TQ:2 * TQ])
    return pltpu.bitcast(jnp.concatenate(parts, axis=0), bf16)


def _head(ref, h, c0, n):
    r = h * (DH // 2)
    if not isinstance(r, int):
        r = pl.multiple_of(r, DH // 2)
    return pltpu.bitcast(ref[pl.ds(r, DH // 2), c0:c0 + n], bf16)


def _kernel(x_hbm, wqkv_hbm, wo_hbm, win_hbm, wsp_hbm, bsp_hbm, wout_hbm, c_hbm, wmod_hbm,
            out_hbm,
            x_v, wqkv_v, wo_v, win_v, wsp_v, wout_v, wmod_v,
            wqT_v, wvT_v, h_v, k_v, kf_v, qT_v, qf_v, vT_v, oT_v,
            kb0, kb1, kr_v, p0, p1, l0, l1, bad_v, sf_v,
            x1_v, z1_v, z2_v, bcol_v, mod_v, out_v, bsp_v, c_v,
            sems, xsems, osems):
    copies = {
        "c": (c_hbm, c_v),
        "wmod0": (wmod_hbm.at[:, 0:2 * D], wmod_v.at[:, 0:2 * D]),
        "wk": (wqkv_hbm.at[:, D:2 * D], wqkv_v.at[:, D:2 * D]),
        "wq": (wqkv_hbm.at[:, 0:D], wqkv_v.at[:, 0:D]),
        "wv": (wqkv_hbm.at[:, 2 * D:3 * D], wqkv_v.at[:, 2 * D:3 * D]),
        "wmod1": (wmod_hbm.at[:, 2 * D:6 * D], wmod_v.at[:, 2 * D:6 * D]),
        "bsp": (bsp_hbm, bsp_v),
        "wo": (wo_hbm, wo_v),
        "win": (win_hbm, win_v),
        "wout": (wout_hbm, wout_v),
        "wsp": (wsp_hbm, wsp_v),
    }
    cp = {name: pltpu.make_async_copy(src, dst, sems.at[i])
          for i, (name, (src, dst)) in enumerate(copies.items())}

    def x_copy(i):
        r = pl.multiple_of(i * TA, TA)
        return pltpu.make_async_copy(x_hbm.at[pl.ds(r, TA), :], x_v.at[pl.ds(r, TA), :], xsems.at[i])

    cp["c"].start()
    x_copy(0).start()
    cp["wmod0"].start()

    cp["c"].wait()
    cf = c_v[...].astype(f32)
    sc8 = jnp.broadcast_to((cf * jax.nn.sigmoid(cf)).astype(bf16), (8, D))
    x_copy(0).wait()
    cp["wk"].start()
    n0 = _ln(x_v[0:TA // 2, :].astype(f32))
    cp["wmod0"].wait()
    x_copy(1).start()
    x_copy(2).start()
    mod_v[:, 0:2 * D] = jnp.dot(sc8, wmod_v[:, 0:2 * D], preferred_element_type=f32)

    TH = TA // 2

    def a_ln(j, n=None):
        r = pl.multiple_of(j * TH, TH)
        if n is None:
            n = _ln(x_v[pl.ds(r, TH), :].astype(f32))
        h = (n * (1.0 + mod_v[0:1, D:2 * D]) + mod_v[0:1, 0:D]).astype(bf16)
        h_v[pl.ds(r, TH), :] = h
        return h

    def a_k(j, h):
        kk = jnp.dot(h, wqkv_v[:, D:2 * D], preferred_element_type=f32)
        k_v[pl.ds(pl.multiple_of(j * (TH // 2), TH // 2), TH // 2), :] = pltpu.bitcast(kk.astype(bf16), u32)
        kf_v[pl.ds(pl.multiple_of(j * TH, TH), TH), :] = kk

    h0 = a_ln(0, n0)
    cp["wk"].wait()

    def phase_a1(i, h):
        @pl.when(i + 3 < NA)
        def _():
            x_copy(i + 3).start()

        @pl.when(i == 3)
        def _():
            cp["wq"].start()
            cp["wv"].start()
        x_copy(i + 1).wait()
        hb = a_ln(2 * i + 1)
        a_k(2 * i, h)
        hn = a_ln(2 * i + 2)
        a_k(2 * i + 1, hb)
        return hn
    hl = lax.fori_loop(0, NA - 1, phase_a1, h0)
    cp["wq"].wait()
    cp["wv"].wait()
    for name in ("wmod1", "bsp", "wo", "win", "wout", "wsp"):
        cp[name].start()
    hb = a_ln(2 * NA - 1)
    a_k(2 * NA - 2, hl)
    a_k(2 * NA - 1, hb)
    wqT_v[...] = wqkv_v[:, 0:D].T
    wvT_v[...] = wqkv_v[:, 2 * D:3 * D].T

    def phase_a2(i, vm):
        r = pl.multiple_of(i * TA2, TA2)
        ht = h_v[pl.ds(r, TA2), :]
        qT = lax.dot_general(wqT_v[...], ht, NT, preferred_element_type=f32) * QSCALE
        qf_v[:, :, pl.ds(r, TA2)] = qT.reshape(H, DH, TA2)
        qT_v[:, pl.ds(r, TA2)] = pltpu.bitcast(qT.astype(bf16), u32)
        vT = lax.dot_general(wvT_v[...], ht, NT, preferred_element_type=f32)
        vT_v[:, pl.ds(r, TA2)] = pltpu.bitcast(vT.astype(bf16), u32)
        rh = pl.multiple_of(i * (TA2 // 2), TA2 // 2)
        for g in range(H // 8):
            kg = k_v[pl.ds(rh, TA2 // 2), g * 128:(g + 1) * 128]
            for j in range(8):
                kr_v[g * 8 + j, pl.ds(rh, TA2 // 2), :] = kg if j == 0 else pltpu.roll(kg, 128 - j * DH, 1)
        va = jnp.abs(vT).reshape(D // 8, 8, TA2).max(axis=0)
        for j in range(TA2 // 128):
            vm = jnp.maximum(vm, va[:, j * 128:(j + 1) * 128])
        return vm
    vmax = lax.fori_loop(0, S // TA2, phase_a2, jnp.zeros((8, 128), f32), unroll=2)
    bad_v[...] = jnp.where(vmax <= V_MAX, 0.0, 1.0)

    def build_k(h, kb):
        gl = pl.multiple_of((h // 8) * 128, 128)
        sh = (128 - (h % 8) * DH) % 128
        kk = jnp.concatenate([kf_v[st + ma + mb:st + ma + mb + v, pl.ds(gl, 128)]
                              for (st, ma, mb, v) in SEGS if v], axis=0)
        kk = pltpu.roll(kk, sh, 1)
        for d in range(DH):
            kb[d] = jnp.broadcast_to(kk[:, d:d + 1], (SV, 128))

    def block(u, hp, hc, p_rd, p_wr, l_rd, l_wr, kb_rd, use_vpu, bad):
        consume = hc is not None
        q0 = u * TQ
        qw = _head(qT_v, hp, q0, TQ)
        l = [None] * NL
        acc = None
        npv = 0
        units = {}

        def ladd(li, t):
            l[li] = t if l[li] is None else l[li] + t

        def put(n, val):
            units[n] = val
            if n ^ 1 in units:
                _p_store(p_wr, u, n // 2, units.pop(n & ~1), units.pop(n | 1))

        def vpu8(o):
            cc = [None] * NCH
            for d in range(DH):
                t = kb_rd[d, o:o + 8, :] * jnp.broadcast_to(qf_v[hp, d:d + 1, q0:q0 + TQ], (8, TQ))
                cc[d % NCH] = t if cc[d % NCH] is None else cc[d % NCH] + t
            return jnp.exp2(sum(cc[1:], cc[0]))

        def qk(a, b, li):
            kk = pltpu.bitcast(kr_v[hp, a // 2:b // 2, :], bf16)[:, 0:DH]
            p = jnp.exp2(jnp.dot(kk, qw, preferred_element_type=f32))
            for r in range((b - a) // 16):
                ladd(li, p[r * 16:r * 16 + 8] + p[r * 16 + 8:r * 16 + 16])
            for r in range((b - a) // 16):
                put(a // 16 + r, p[r * 16:(r + 1) * 16])

        for i, (st, ma, mb, v) in enumerate(SEGS):
            end = st + ma + mb + v
            if use_vpu and v:
                la = (2 * i) % NL
                lb = (2 * i + 1) % NL
                e0 = vpu8(i * SEG_V)
                ladd(la, e0)
                qk(st, st + ma, la)
                e1 = vpu8(i * SEG_V + 8)
                ladd(lb, e1)
                put((end - v) // 16, jnp.concatenate([e0, e1], axis=0))
                qk(st + ma, st + ma + mb, lb)
            else:
                qk(st, end, (2 * i) % NL)
            while consume and (npv + 1) * PVK <= end:
                k0 = npv * PVK
                t = jnp.dot(_head(vT_v, hc, k0, PVK), _p_load(p_rd, u, k0, PVK), preferred_element_type=f32)
                acc = t if acc is None else acc + t
                npv += 1
        if consume:
            ls = l_rd[:, q0:q0 + TQ].sum(axis=0, keepdims=True)
            oT_v[pl.ds(pl.multiple_of(hc * DH, DH), DH), q0:q0 + TQ] = (acc * (1.0 / ls)).astype(bf16)
            bad = jnp.where((ls >= L_LO) & (ls <= L_HI), bad, 1.0)
        l_wr[:, q0:q0 + TQ] = sum(l[1:], l[0])
        return bad

    def mod_rest(j):
        c0 = 2 * D + j * 128
        mod_v[:, c0:c0 + 128] = jnp.dot(sc8, wmod_v[:, c0:c0 + 128], preferred_element_type=f32)
        bj = jnp.broadcast_to(bsp_v[...].astype(f32).reshape(1, S)[:, j * 128:(j + 1) * 128], (128, 128))
        bcol_v[j * 128:(j + 1) * 128, :] = bj.T

    def step(h, p_rd, p_wr, l_rd, l_wr, kb_rd, kb_wr, first=False):
        bad = None if first else bad_v[...]
        for u in range(NQ):
            if first:
                mod_rest(u)
            bad = block(u, h + 1, None if first else h, p_rd, p_wr, l_rd, l_wr, kb_rd, not first, bad)
        if not first:
            bad_v[...] = bad
        build_k(jnp.minimum(h + 2, H - 1), kb_wr)

    cp["wmod1"].wait()
    cp["bsp"].wait()
    step(-1, None, p0, None, l0, kb0, kb1, first=True)

    def phase_b(h, carry):
        lax.cond(h % 2 == 0,
                 lambda: step(h, p0, p1, l0, l1, kb1, kb0),
                 lambda: step(h, p1, p0, l1, l0, kb0, kb1))
        return carry
    lax.fori_loop(0, H - 1, phase_b, 0)
    lsl = l1[...].sum(axis=0, keepdims=True)
    badl = jnp.where((lsl >= L_LO) & (lsl <= L_HI), 0.0, 1.0)
    bad = bad_v[...]
    for j in range(NQ):
        bad = jnp.maximum(bad, badl[:, j * TQ:(j + 1) * TQ])

    @pl.when(jnp.max(bad) > 0.0)
    def _():
        row = lax.broadcasted_iota(jnp.int32, (128, TF), 0) // DH

        def exact(b, carry):
            h = b // (S // TF)
            q0 = pl.multiple_of((b % (S // TF)) * TF, TF)
            ub = (b % (S // TF)) * (TF // TQ)
            g = h // 8
            gl = pl.multiple_of(g * 128, 128)
            qg = qf_v[pl.ds(g * 8, 8), :, pl.ds(q0, TF)].reshape(128, TF)
            qw = jnp.where(row == h % 8, qg, 0.0).astype(bf16)
            mx = jnp.full((8, TF), -jnp.inf, f32)
            for c in range(S // TK):
                kk = pltpu.bitcast(k_v[c * TK // 2:(c + 1) * TK // 2, pl.ds(gl, 128)], bf16)
                s = jnp.dot(kk, qw, preferred_element_type=f32)
                sf_v[c * TK:(c + 1) * TK, :] = s
                mx = jnp.maximum(mx, s.reshape(TK // 8, 8, TF).max(axis=0))
            m = mx.max(axis=0, keepdims=True)
            l = jnp.zeros((8, TF), f32)
            acc = jnp.zeros((DH, TF), f32)
            for c in range(S // TK):
                p = jnp.exp2(sf_v[c * TK:(c + 1) * TK, :] - m)
                l = l + p.reshape(TK // 8, 8, TF).sum(axis=0)
                for j in range(TF // TQ):
                    for t in range(TK // 32):
                        _p_store(p1, ub + j, c * (TK // 32) + t, p[t * 32:t * 32 + 16, j * TQ:(j + 1) * TQ],
                                 p[t * 32 + 16:t * 32 + 32, j * TQ:(j + 1) * TQ])
                acc = acc + jnp.dot(_head(vT_v, h, c * TK, TK), p.astype(bf16),
                                    preferred_element_type=f32)
            l1[:, pl.ds(q0, TF)] = l
            o = acc / l.sum(axis=0, keepdims=True)
            oT_v[pl.ds(pl.multiple_of(h * DH, DH), DH), pl.ds(q0, TF)] = o.astype(bf16)
            return carry
        lax.fori_loop(0, H * (S // TF), exact, 0)

    cp["wo"].wait()
    cp["win"].wait()

    def c_s1(i):
        r = pl.multiple_of(i * TC, TC)
        y = lax.dot_general(oT_v[:, pl.ds(r, TC)], wo_v[...], TN, preferred_element_type=f32)
        x1 = x_v[pl.ds(r, TC), :].astype(f32) + mod_v[0:1, 2 * D:3 * D] * y
        x1_v[pl.ds(r, TC), :] = x1
        return (_ln(x1) * (1.0 + mod_v[0:1, 4 * D:5 * D]) + mod_v[0:1, 3 * D:4 * D]).astype(bf16)

    def c_z2(i, h2):
        r = pl.multiple_of(i * TC, TC)
        for a in range(0, TC, TC // 2):
            z2 = _gelu(jnp.dot(h2[a:a + TC // 2], win_v[:, FH:F], preferred_element_type=f32))
            z2_v[pl.ds(r + a, TC // 2), :] = _ln(z2).astype(bf16)

    def c_z1(i, h2):
        r = pl.multiple_of(i * TC, TC)
        z1_v[pl.ds(r, TC), :] = jnp.dot(h2, win_v[:, 0:FH], preferred_element_type=f32).astype(bf16)

    def last_pv(u):
        q0 = u * TQ if isinstance(u, int) else pl.multiple_of(u * TQ, TQ)
        acc = None
        for c in range(S // PVK):
            k0 = c * PVK
            t = jnp.dot(_head(vT_v, H - 1, k0, PVK), _p_load(p1, u, k0, PVK), preferred_element_type=f32)
            acc = t if acc is None else acc + t
        ls = l1[:, pl.ds(q0, TQ)].sum(axis=0, keepdims=True)
        oT_v[(H - 1) * DH:H * DH, pl.ds(q0, TQ)] = (acc * (1.0 / ls)).astype(bf16)

    last_pv(0)
    last_pv(1)
    h20 = c_s1(0)
    for u in range(2, NPRE):
        last_pv(u)

    def phase_c(i, h2):
        c_z2(i, h2)
        hn = c_s1(i + 1)
        c_z1(i, h2)
        last_pv(jnp.minimum(NPRE + i, NQ - 1))
        return hn
    h2 = lax.fori_loop(0, S // TC - 1, phase_c, h20)
    c_z2(S // TC - 1, h2)
    c_z1(S // TC - 1, h2)

    cp["wsp"].wait()
    cp["wout"].wait()

    TO = TD // 2

    def out_copy(j):
        r = pl.multiple_of(j * TO, TO)
        return pltpu.make_async_copy(out_v.at[pl.ds(r, TO), :], out_hbm.at[pl.ds(r, TO), :], osems.at[j])

    def phase_d(i, carry):
        r = pl.multiple_of(i * TD, TD)
        g = jnp.dot(wsp_v[pl.ds(r, TD), :], z2_v[...], preferred_element_type=f32)
        g = g + jnp.concatenate([bcol_v[pl.ds(r, TD), :]] * (FH // 128), axis=1)
        u = (_gelu(z1_v[pl.ds(r, TD), :].astype(f32)) * g).astype(bf16)
        for a in range(2):
            ra = pl.multiple_of(r + a * TO, TO)
            y2 = jnp.dot(u[a * TO:(a + 1) * TO], wout_v[...], preferred_element_type=f32)
            out_v[pl.ds(ra, TO), :] = (x1_v[pl.ds(ra, TO), :] + mod_v[0:1, 5 * D:6 * D] * y2).astype(bf16)
            out_copy(2 * i + a).start()
        return carry
    lax.fori_loop(0, S // TD, phase_d, 0, unroll=2)
    for j in range(S // TO):
        out_copy(j).wait()


@jax.jit
def pallas_adaLN_cond__softmax_full_mha__mixer_gmlp__prompt_kernel(
    A_x: jax.Array,
    A_wqkv: jax.Array,
    A_wo: jax.Array,
    B_x: jax.Array,
    B_w_in: jax.Array,
    B_w_sp: jax.Array,
    B_b_sp: jax.Array,
    B_w_out: jax.Array,
    c: jax.Array,
    w_mod: jax.Array,
):
    del B_x
    any_spec = pl.BlockSpec(memory_space=pl.ANY)
    out = pl.pallas_call(
        _kernel,
        out_shape=jax.ShapeDtypeStruct((S, D), bf16),
        in_specs=[any_spec] * 9,
        out_specs=any_spec,
        scratch_shapes=[
            pltpu.VMEM((S, D), bf16),
            pltpu.VMEM((D, 3 * D), bf16),
            pltpu.VMEM((D, D), bf16),
            pltpu.VMEM((D, F), bf16),
            pltpu.VMEM((S, S), bf16),
            pltpu.VMEM((FH, D), bf16),
            pltpu.VMEM((D, 6 * D), bf16),
            pltpu.VMEM((D, D), bf16),
            pltpu.VMEM((D, D), bf16),
            pltpu.VMEM((S, D), bf16),
            pltpu.VMEM((S // 2, D), u32),
            pltpu.VMEM((S, D), f32),
            pltpu.VMEM((D // 2, S), u32),
            pltpu.VMEM((H, DH, S), f32),
            pltpu.VMEM((D // 2, S), u32),
            pltpu.VMEM((D, S), bf16),
            pltpu.VMEM((DH, SV, 128), f32),
            pltpu.VMEM((DH, SV, 128), f32),
            pltpu.VMEM((H, S // 2, 128), u32),
            pltpu.VMEM((NQ * S // 4, 2 * TQ), u32),
            pltpu.VMEM((NQ * S // 4, 2 * TQ), u32),
            pltpu.VMEM((8, S), f32),
            pltpu.VMEM((8, S), f32),
            pltpu.VMEM((8, TQ), f32),
            pltpu.VMEM((S, TF), f32),
            pltpu.VMEM((S, D), f32),
            pltpu.VMEM((S, FH), bf16),
            pltpu.VMEM((S, FH), bf16),
            pltpu.VMEM((S, 128), f32),
            pltpu.VMEM((8, 6 * D), f32),
            pltpu.VMEM((S, D), bf16),
            pltpu.VMEM((S,), bf16),
            pltpu.VMEM((1, D), bf16),
            pltpu.SemaphoreType.DMA((11,)),
            pltpu.SemaphoreType.DMA((NA,)),
            pltpu.SemaphoreType.DMA((2 * S // TD,)),
        ],
        compiler_params=pltpu.CompilerParams(vmem_limit_bytes=120 * 2 ** 20),
    )(A_x.reshape(S, D), A_wqkv, A_wo, B_w_in, B_w_sp, B_b_sp, B_w_out, c, w_mod)
    return out.reshape(1, S, D)
```

```python
import math

import jax
import jax.numpy as jnp
from jax import lax
import jax.experimental.pallas as pl
import jax.experimental.pallas.tpu as pltpu

S = 2048
D = 512
H = 32
DH = 16
F = 1792
FH = 896
EPS = 1e-5
bf16 = jnp.bfloat16
f32 = jnp.float32
u32 = jnp.uint32

TQ = 128
NQ = S // TQ
SEG_V = 16
_PAT = [(48, 48), (48, 32), (48, 32)]
SEGS = []
_st = 0
while _st < S:
    _ma, _mb = _PAT[len(SEGS) % len(_PAT)]
    if _st + _ma + _mb + SEG_V > S:
        SEGS.append((_st, S - _st, 0, 0))
        _st = S
    else:
        SEGS.append((_st, _ma, _mb, SEG_V))
        _st += _ma + _mb + SEG_V
SV = sum(seg[3] for seg in SEGS)
PVK = 128
NCH = 2
NL = 3
NPRE = 10
TK = 128
TF = 256
TA = 256
TA2 = 512
TC = 256
TD = 256
NA = S // TA
QSCALE = (DH ** -0.5) * math.log2(math.e)
L_LO = 2.0 ** -80
L_HI = 2.0 ** 100
V_MAX = 2.0 ** 20
NT = (((1,), (1,)), ((), ()))
TN = (((0,), (0,)), ((), ()))


def _ln(x):
    m = jnp.mean(x, axis=-1, keepdims=True)
    xc = x - m
    v = jnp.mean(xc * xc, axis=-1, keepdims=True)
    return xc * lax.rsqrt(v + EPS)


def _gelu(x):
    c = math.sqrt(2.0 / math.pi)
    return 0.5 * x * (1.0 + jnp.tanh(c * (x + 0.044715 * (x * x * x))))


def _p_store(p_ref, u, pair, ua, ub):
    r = u * (S // 4) + pair * 8
    if not isinstance(r, int):
        r = pl.multiple_of(r, 8)
    both = jnp.concatenate([ua, ub], axis=1).astype(bf16)
    p_ref[pl.ds(r, 8), :] = pltpu.bitcast(both, u32)


def _p_load(p_ref, u, k0, n):
    r = u * (S // 4) + k0 // 4
    if not isinstance(r, int):
        r = pl.multiple_of(r, 8)
    w = p_ref[pl.ds(r, n // 4), :]
    parts = []
    for t in range(n // 32):
        parts.append(w[t * 8:(t + 1) * 8, 0:TQ])
        parts.append(w[t * 8:(t + 1) * 8, TQ:2 * TQ])
    return pltpu.bitcast(jnp.concatenate(parts, axis=0), bf16)


def _head(ref, h, c0, n):
    r = h * (DH // 2)
    if not isinstance(r, int):
        r = pl.multiple_of(r, DH // 2)
    return pltpu.bitcast(ref[pl.ds(r, DH // 2), pl.ds(c0, n)], bf16)


def _kernel(x_hbm, wqkv_hbm, wo_hbm, win_hbm, wsp_hbm, bsp_hbm, wout_hbm, c_hbm, wmod_hbm,
            out_hbm,
            x_v, wqkv_v, wo_v, win_v, wsp_v, wout_v, wmod_v,
            wqT_v, wvT_v, h_v, k_v, kf_v, qT_v, qf_v, vT_v, oT_v,
            kb0, kb1, kr_v, p0, p1, l0, l1, bad_v, sf_v,
            x1_v, z1_v, z2_v, bcol_v, mod_v, out_v, bsp_v, c_v,
            sems, xsems, osems):
    copies = {
        "c": (c_hbm, c_v),
        "wmod0": (wmod_hbm.at[:, 0:2 * D], wmod_v.at[:, 0:2 * D]),
        "wk": (wqkv_hbm.at[:, D:2 * D], wqkv_v.at[:, D:2 * D]),
        "wq": (wqkv_hbm.at[:, 0:D], wqkv_v.at[:, 0:D]),
        "wv": (wqkv_hbm.at[:, 2 * D:3 * D], wqkv_v.at[:, 2 * D:3 * D]),
        "wmod1": (wmod_hbm.at[:, 2 * D:6 * D], wmod_v.at[:, 2 * D:6 * D]),
        "bsp": (bsp_hbm, bsp_v),
        "wo": (wo_hbm, wo_v),
        "win": (win_hbm, win_v),
        "wout": (wout_hbm, wout_v),
        "wsp": (wsp_hbm, wsp_v),
    }
    cp = {name: pltpu.make_async_copy(src, dst, sems.at[i])
          for i, (name, (src, dst)) in enumerate(copies.items())}

    def x_copy(i):
        r = pl.multiple_of(i * TA, TA)
        return pltpu.make_async_copy(x_hbm.at[pl.ds(r, TA), :], x_v.at[pl.ds(r, TA), :], xsems.at[i])

    cp["c"].start()
    x_copy(0).start()
    cp["wmod0"].start()

    cp["c"].wait()
    cf = c_v[...].astype(f32)
    sc8 = jnp.broadcast_to((cf * jax.nn.sigmoid(cf)).astype(bf16), (8, D))
    x_copy(0).wait()
    cp["wk"].start()
    n0 = _ln(x_v[0:TA // 2, :].astype(f32))
    cp["wmod0"].wait()
    x_copy(1).start()
    x_copy(2).start()
    mod_v[:, 0:2 * D] = jnp.dot(sc8, wmod_v[:, 0:2 * D], preferred_element_type=f32)

    TH = TA // 2

    def a_ln(j, n=None):
        r = pl.multiple_of(j * TH, TH)
        if n is None:
            n = _ln(x_v[pl.ds(r, TH), :].astype(f32))
        h = (n * (1.0 + mod_v[0:1, D:2 * D]) + mod_v[0:1, 0:D]).astype(bf16)
        h_v[pl.ds(r, TH), :] = h
        return h

    def a_k(j, h):
        kk = jnp.dot(h, wqkv_v[:, D:2 * D], preferred_element_type=f32)
        k_v[pl.ds(pl.multiple_of(j * (TH // 2), TH // 2), TH // 2), :] = pltpu.bitcast(kk.astype(bf16), u32)
        kf_v[pl.ds(pl.multiple_of(j * TH, TH), TH), :] = kk

    h0 = a_ln(0, n0)
    cp["wk"].wait()

    def phase_a1(i, h):
        @pl.when(i + 3 < NA)
        def _():
            x_copy(i + 3).start()

        @pl.when(i == 3)
        def _():
            cp["wq"].start()
            cp["wv"].start()
        x_copy(i + 1).wait()
        hb = a_ln(2 * i + 1)
        a_k(2 * i, h)
        hn = a_ln(2 * i + 2)
        a_k(2 * i + 1, hb)
        return hn
    hl = lax.fori_loop(0, NA - 1, phase_a1, h0)
    cp["wq"].wait()
    cp["wv"].wait()
    for name in ("wmod1", "bsp", "wo", "win", "wout", "wsp"):
        cp[name].start()
    hb = a_ln(2 * NA - 1)
    a_k(2 * NA - 2, hl)
    a_k(2 * NA - 1, hb)
    wqT_v[...] = wqkv_v[:, 0:D].T
    wvT_v[...] = wqkv_v[:, 2 * D:3 * D].T

    def phase_a2(i, vm):
        r = pl.multiple_of(i * TA2, TA2)
        ht = h_v[pl.ds(r, TA2), :]
        qT = lax.dot_general(wqT_v[...], ht, NT, preferred_element_type=f32) * QSCALE
        qf_v[:, :, pl.ds(r, TA2)] = qT.reshape(H, DH, TA2)
        qT_v[:, pl.ds(r, TA2)] = pltpu.bitcast(qT.astype(bf16), u32)
        vT = lax.dot_general(wvT_v[...], ht, NT, preferred_element_type=f32)
        vT_v[:, pl.ds(r, TA2)] = pltpu.bitcast(vT.astype(bf16), u32)
        rh = pl.multiple_of(i * (TA2 // 2), TA2 // 2)
        for g in range(H // 8):
            kg = k_v[pl.ds(rh, TA2 // 2), g * 128:(g + 1) * 128]
            for j in range(8):
                kr_v[g * 8 + j, pl.ds(rh, TA2 // 2), :] = kg if j == 0 else pltpu.roll(kg, 128 - j * DH, 1)
        va = jnp.abs(vT).reshape(D // 8, 8, TA2).max(axis=0)
        for j in range(TA2 // 128):
            vm = jnp.maximum(vm, va[:, j * 128:(j + 1) * 128])
        return vm
    vmax = lax.fori_loop(0, S // TA2, phase_a2, jnp.zeros((8, 128), f32), unroll=2)
    bad_v[...] = jnp.where(vmax <= V_MAX, 0.0, 1.0)

    def build_k(h, kb):
        gl = pl.multiple_of((h // 8) * 128, 128)
        sh = (128 - (h % 8) * DH) % 128
        kk = jnp.concatenate([kf_v[st + ma + mb:st + ma + mb + v, pl.ds(gl, 128)]
                              for (st, ma, mb, v) in SEGS if v], axis=0)
        kk = pltpu.roll(kk, sh, 1)
        for d in range(DH):
            kb[d] = jnp.broadcast_to(kk[:, d:d + 1], (SV, 128))

    def block(u, hp, hc, p_rd, p_wr, l_rd, l_wr, kb_rd, use_vpu, bad):
        consume = hc is not None
        q0 = u * TQ
        qw = _head(qT_v, hp, q0, TQ)
        l = [None] * NL
        acc = None
        npv = 0
        units = {}

        def ladd(li, t):
            l[li] = t if l[li] is None else l[li] + t

        def put(n, val):
            units[n] = val
            if n ^ 1 in units:
                _p_store(p_wr, u, n // 2, units.pop(n & ~1), units.pop(n | 1))

        def vpu8(o):
            cc = [None] * NCH
            for d in range(DH):
                t = kb_rd[d, o:o + 8, :] * jnp.broadcast_to(qf_v[hp, d:d + 1, q0:q0 + TQ], (8, TQ))
                cc[d % NCH] = t if cc[d % NCH] is None else cc[d % NCH] + t
            return jnp.exp2(sum(cc[1:], cc[0]))

        def qk(a, b, li):
            kk = pltpu.bitcast(kr_v[hp, a // 2:b // 2, :], bf16)[:, 0:DH]
            p = jnp.exp2(jnp.dot(kk, qw, preferred_element_type=f32))
            for r in range((b - a) // 16):
                ladd(li, p[r * 16:r * 16 + 8] + p[r * 16 + 8:r * 16 + 16])
            for r in range((b - a) // 16):
                put(a // 16 + r, p[r * 16:(r + 1) * 16])

        for i, (st, ma, mb, v) in enumerate(SEGS):
            end = st + ma + mb + v
            if use_vpu and v:
                la = (2 * i) % NL
                lb = (2 * i + 1) % NL
                e0 = vpu8(i * SEG_V)
                ladd(la, e0)
                qk(st, st + ma, la)
                e1 = vpu8(i * SEG_V + 8)
                ladd(lb, e1)
                put((end - v) // 16, jnp.concatenate([e0, e1], axis=0))
                qk(st + ma, st + ma + mb, lb)
            else:
                qk(st, end, (2 * i) % NL)
            while consume and (npv + 1) * PVK <= end:
                k0 = npv * PVK
                t = jnp.dot(_head(vT_v, hc, k0, PVK), _p_load(p_rd, u, k0, PVK), preferred_element_type=f32)
                acc = t if acc is None else acc + t
                npv += 1
        if consume:
            ls = l_rd[:, q0:q0 + TQ].sum(axis=0, keepdims=True)
            oT_v[pl.ds(pl.multiple_of(hc * DH, DH), DH), q0:q0 + TQ] = (acc * (1.0 / ls)).astype(bf16)
            bad = jnp.where((ls >= L_LO) & (ls <= L_HI), bad, 1.0)
        l_wr[:, q0:q0 + TQ] = sum(l[1:], l[0])
        return bad

    def mod_rest(j):
        c0 = 2 * D + j * 128
        mod_v[:, c0:c0 + 128] = jnp.dot(sc8, wmod_v[:, c0:c0 + 128], preferred_element_type=f32)
        bj = jnp.broadcast_to(bsp_v[...].astype(f32).reshape(1, S)[:, j * 128:(j + 1) * 128], (128, 128))
        bcol_v[j * 128:(j + 1) * 128, :] = bj.T

    def step(h, p_rd, p_wr, l_rd, l_wr, kb_rd, kb_wr, first=False):
        bad = None if first else bad_v[...]
        for u in range(NQ):
            if first:
                mod_rest(u)
            bad = block(u, h + 1, None if first else h, p_rd, p_wr, l_rd, l_wr, kb_rd, not first, bad)
        if not first:
            bad_v[...] = bad
        build_k(jnp.minimum(h + 2, H - 1), kb_wr)

    cp["wmod1"].wait()
    cp["bsp"].wait()
    step(-1, None, p0, None, l0, kb0, kb1, first=True)

    def phase_b(h, carry):
        lax.cond(h % 2 == 0,
                 lambda: step(h, p0, p1, l0, l1, kb1, kb0),
                 lambda: step(h, p1, p0, l1, l0, kb0, kb1))
        return carry
    lax.fori_loop(0, H - 1, phase_b, 0)
    lsl = l1[...].sum(axis=0, keepdims=True)
    badl = jnp.where((lsl >= L_LO) & (lsl <= L_HI), 0.0, 1.0)
    bad = bad_v[...]
    for j in range(NQ):
        bad = jnp.maximum(bad, badl[:, j * TQ:(j + 1) * TQ])

    @pl.when(jnp.max(bad) > 0.0)
    def _():
        def exact(b, carry):
            h = b // (S // TF)
            q0 = pl.multiple_of((b % (S // TF)) * TF, TF)
            ub = (b % (S // TF)) * (TF // TQ)
            qw = _head(qT_v, h, q0, TF)
            mx = jnp.full((8, TF), -jnp.inf, f32)
            for c in range(S // TK):
                kk = pltpu.bitcast(kr_v[h, c * TK // 2:(c + 1) * TK // 2, :], bf16)[:, 0:DH]
                s = jnp.dot(kk, qw, preferred_element_type=f32)
                sf_v[c * TK:(c + 1) * TK, :] = s
                mx = jnp.maximum(mx, s.reshape(TK // 8, 8, TF).max(axis=0))
            m = mx.max(axis=0, keepdims=True)
            l = jnp.zeros((8, TF), f32)
            acc = jnp.zeros((DH, TF), f32)
            for c in range(S // TK):
                p = jnp.exp2(sf_v[c * TK:(c + 1) * TK, :] - m)
                l = l + p.reshape(TK // 8, 8, TF).sum(axis=0)
                for j in range(TF // TQ):
                    for t in range(TK // 32):
                        _p_store(p1, ub + j, c * (TK // 32) + t, p[t * 32:t * 32 + 16, j * TQ:(j + 1) * TQ],
                                 p[t * 32 + 16:t * 32 + 32, j * TQ:(j + 1) * TQ])
                acc = acc + jnp.dot(_head(vT_v, h, c * TK, TK), p.astype(bf16),
                                    preferred_element_type=f32)
            l1[:, pl.ds(q0, TF)] = l
            o = acc / l.sum(axis=0, keepdims=True)
            oT_v[pl.ds(pl.multiple_of(h * DH, DH), DH), pl.ds(q0, TF)] = o.astype(bf16)
            return carry
        lax.fori_loop(0, H * (S // TF), exact, 0)

    cp["wo"].wait()
    cp["win"].wait()

    def c_s1(i):
        r = pl.multiple_of(i * TC, TC)
        y = lax.dot_general(oT_v[:, pl.ds(r, TC)], wo_v[...], TN, preferred_element_type=f32)
        x1 = x_v[pl.ds(r, TC), :].astype(f32) + mod_v[0:1, 2 * D:3 * D] * y
        x1_v[pl.ds(r, TC), :] = x1
        return (_ln(x1) * (1.0 + mod_v[0:1, 4 * D:5 * D]) + mod_v[0:1, 3 * D:4 * D]).astype(bf16)

    def c_z2(i, h2):
        r = pl.multiple_of(i * TC, TC)
        for a in range(0, TC, TC // 2):
            z2 = _gelu(jnp.dot(h2[a:a + TC // 2], win_v[:, FH:F], preferred_element_type=f32))
            z2_v[pl.ds(r + a, TC // 2), :] = _ln(z2).astype(bf16)

    def c_z1(i, h2):
        r = pl.multiple_of(i * TC, TC)
        z1_v[pl.ds(r, TC), :] = jnp.dot(h2, win_v[:, 0:FH], preferred_element_type=f32).astype(bf16)

    def last_pv(u):
        q0 = u * TQ if isinstance(u, int) else pl.multiple_of(u * TQ, TQ)
        acc = None
        for c in range(S // PVK):
            k0 = c * PVK
            t = jnp.dot(_head(vT_v, H - 1, k0, PVK), _p_load(p1, u, k0, PVK), preferred_element_type=f32)
            acc = t if acc is None else acc + t
        ls = l1[:, pl.ds(q0, TQ)].sum(axis=0, keepdims=True)
        oT_v[(H - 1) * DH:H * DH, pl.ds(q0, TQ)] = (acc * (1.0 / ls)).astype(bf16)

    last_pv(0)
    last_pv(1)
    h20 = c_s1(0)
    for u in range(2, NPRE):
        last_pv(u)

    def phase_c(i, h2):
        c_z2(i, h2)
        hn = c_s1(i + 1)
        c_z1(i, h2)
        last_pv(jnp.minimum(NPRE + i, NQ - 1))
        return hn
    h2 = lax.fori_loop(0, S // TC - 1, phase_c, h20)
    c_z2(S // TC - 1, h2)
    c_z1(S // TC - 1, h2)

    cp["wsp"].wait()
    cp["wout"].wait()

    TO = TD // 2

    def out_copy(j):
        r = pl.multiple_of(j * TO, TO)
        return pltpu.make_async_copy(out_v.at[pl.ds(r, TO), :], out_hbm.at[pl.ds(r, TO), :], osems.at[j])

    def phase_d(i, carry):
        r = pl.multiple_of(i * TD, TD)
        g = jnp.dot(wsp_v[pl.ds(r, TD), :], z2_v[...], preferred_element_type=f32)
        g = g + jnp.concatenate([bcol_v[pl.ds(r, TD), :]] * (FH // 128), axis=1)
        u = (_gelu(z1_v[pl.ds(r, TD), :].astype(f32)) * g).astype(bf16)
        for a in range(2):
            ra = pl.multiple_of(r + a * TO, TO)
            y2 = jnp.dot(u[a * TO:(a + 1) * TO], wout_v[...], preferred_element_type=f32)
            out_v[pl.ds(ra, TO), :] = (x1_v[pl.ds(ra, TO), :] + mod_v[0:1, 5 * D:6 * D] * y2).astype(bf16)
            out_copy(2 * i + a).start()
        return carry
    lax.fori_loop(0, S // TD, phase_d, 0, unroll=2)
    for j in range(S // TO):
        out_copy(j).wait()


@jax.jit
def pallas_adaLN_cond__softmax_full_mha__mixer_gmlp__prompt_kernel(
    A_x: jax.Array,
    A_wqkv: jax.Array,
    A_wo: jax.Array,
    B_x: jax.Array,
    B_w_in: jax.Array,
    B_w_sp: jax.Array,
    B_b_sp: jax.Array,
    B_w_out: jax.Array,
    c: jax.Array,
    w_mod: jax.Array,
):
    del B_x
    any_spec = pl.BlockSpec(memory_space=pl.ANY)
    out = pl.pallas_call(
        _kernel,
        out_shape=jax.ShapeDtypeStruct((S, D), bf16),
        in_specs=[any_spec] * 9,
        out_specs=any_spec,
        scratch_shapes=[
            pltpu.VMEM((S, D), bf16),
            pltpu.VMEM((D, 3 * D), bf16),
            pltpu.VMEM((D, D), bf16),
            pltpu.VMEM((D, F), bf16),
            pltpu.VMEM((S, S), bf16),
            pltpu.VMEM((FH, D), bf16),
            pltpu.VMEM((D, 6 * D), bf16),
            pltpu.VMEM((D, D), bf16),
            pltpu.VMEM((D, D), bf16),
            pltpu.VMEM((S, D), bf16),
            pltpu.VMEM((S // 2, D), u32),
            pltpu.VMEM((S, D), f32),
            pltpu.VMEM((D // 2, S), u32),
            pltpu.VMEM((H, DH, S), f32),
            pltpu.VMEM((D // 2, S), u32),
            pltpu.VMEM((D, S), bf16),
            pltpu.VMEM((DH, SV, 128), f32),
            pltpu.VMEM((DH, SV, 128), f32),
            pltpu.VMEM((H, S // 2, 128), u32),
            pltpu.VMEM((NQ * S // 4, 2 * TQ), u32),
            pltpu.VMEM((NQ * S // 4, 2 * TQ), u32),
            pltpu.VMEM((8, S), f32),
            pltpu.VMEM((8, S), f32),
            pltpu.VMEM((8, TQ), f32),
            pltpu.VMEM((S, TF), f32),
            pltpu.VMEM((S, D), f32),
            pltpu.VMEM((S, FH), bf16),
            pltpu.VMEM((S, FH), bf16),
            pltpu.VMEM((S, 128), f32),
            pltpu.VMEM((8, 6 * D), f32),
            pltpu.VMEM((S, D), bf16),
            pltpu.VMEM((S,), bf16),
            pltpu.VMEM((1, D), bf16),
            pltpu.SemaphoreType.DMA((11,)),
            pltpu.SemaphoreType.DMA((NA,)),
            pltpu.SemaphoreType.DMA((2 * S // TD,)),
        ],
        compiler_params=pltpu.CompilerParams(vmem_limit_bytes=120 * 2 ** 20),
    )(A_x.reshape(S, D), A_wqkv, A_wo, B_w_in, B_w_sp, B_b_sp, B_w_out, c, w_mod)
    return out.reshape(1, S, D)
```

```python
import math

import jax
import jax.numpy as jnp
from jax import lax
import jax.experimental.pallas as pl
import jax.experimental.pallas.tpu as pltpu

S = 2048
D = 512
H = 32
DH = 16
F = 1792
FH = 896
EPS = 1e-5
bf16 = jnp.bfloat16
f32 = jnp.float32
u32 = jnp.uint32

TQ = 128
NQ = S // TQ
SEG_V = 16
_PAT = [(48, 48), (48, 32), (48, 32)]
SEGS = []
_st = 0
while _st < S:
    _ma, _mb = _PAT[len(SEGS) % len(_PAT)]
    if _st + _ma + _mb + SEG_V > S:
        SEGS.append((_st, S - _st, 0, 0))
        _st = S
    else:
        SEGS.append((_st, _ma, _mb, SEG_V))
        _st += _ma + _mb + SEG_V
SV = sum(seg[3] for seg in SEGS)
PVK = 128
NL = 3
NPRE = 10
TK = 128
TF = 256
TA = 256
TA2 = 512
TC = 256
TD = 256
NA = S // TA
QSCALE = (DH ** -0.5) * math.log2(math.e)
L_LO = 2.0 ** -80
L_HI = 2.0 ** 100
V_MAX = 2.0 ** 20
NT = (((1,), (1,)), ((), ()))
TN = (((0,), (0,)), ((), ()))


def _ln(x):
    m = jnp.mean(x, axis=-1, keepdims=True)
    xc = x - m
    v = jnp.mean(xc * xc, axis=-1, keepdims=True)
    return xc * lax.rsqrt(v + EPS)


def _gelu(x):
    c = math.sqrt(2.0 / math.pi)
    return 0.5 * x * (1.0 + jnp.tanh(c * (x + 0.044715 * (x * x * x))))


def _p_store(p_ref, u, pair, ua, ub):
    r = u * (S // 4) + pair * 8
    if not isinstance(r, int):
        r = pl.multiple_of(r, 8)
    both = jnp.concatenate([ua, ub], axis=1).astype(bf16)
    p_ref[pl.ds(r, 8), :] = pltpu.bitcast(both, u32)


def _p_load(p_ref, u, k0, n):
    r = u * (S // 4) + k0 // 4
    if not isinstance(r, int):
        r = pl.multiple_of(r, 8)
    w = p_ref[pl.ds(r, n // 4), :]
    parts = []
    for t in range(n // 32):
        parts.append(w[t * 8:(t + 1) * 8, 0:TQ])
        parts.append(w[t * 8:(t + 1) * 8, TQ:2 * TQ])
    return pltpu.bitcast(jnp.concatenate(parts, axis=0), bf16)


def _head(ref, h, c0, n):
    r = h * (DH // 2)
    if not isinstance(r, int):
        r = pl.multiple_of(r, DH // 2)
    return pltpu.bitcast(ref[pl.ds(r, DH // 2), pl.ds(c0, n)], bf16)


def _kernel(x_hbm, wqkv_hbm, wo_hbm, win_hbm, wsp_hbm, bsp_hbm, wout_hbm, c_hbm, wmod_hbm,
            out_hbm,
            x_v, wqkv_v, wo_v, win_v, wsp_v, wout_v, wmod_v,
            wqT_v, wvT_v, h_v, k_v, kf_v, qT_v, qf_v, vT_v, oT_v,
            kb0, kb1, kr_v, p0, p1, l0, l1, bad_v, sf_v,
            x1_v, z1_v, z2_v, bcol_v, mod_v, out_v, bsp_v, c_v,
            sems, xsems, osems):
    copies = {
        "c": (c_hbm, c_v),
        "wmod0": (wmod_hbm.at[:, 0:2 * D], wmod_v.at[:, 0:2 * D]),
        "wk": (wqkv_hbm.at[:, D:2 * D], wqkv_v.at[:, D:2 * D]),
        "wq": (wqkv_hbm.at[:, 0:D], wqkv_v.at[:, 0:D]),
        "wv": (wqkv_hbm.at[:, 2 * D:3 * D], wqkv_v.at[:, 2 * D:3 * D]),
        "wmod1": (wmod_hbm.at[:, 2 * D:6 * D], wmod_v.at[:, 2 * D:6 * D]),
        "bsp": (bsp_hbm, bsp_v),
        "wo": (wo_hbm, wo_v),
        "win": (win_hbm, win_v),
        "wout": (wout_hbm, wout_v),
        "wsp": (wsp_hbm, wsp_v),
    }
    cp = {name: pltpu.make_async_copy(src, dst, sems.at[i])
          for i, (name, (src, dst)) in enumerate(copies.items())}

    def x_copy(i):
        r = pl.multiple_of(i * TA, TA)
        return pltpu.make_async_copy(x_hbm.at[pl.ds(r, TA), :], x_v.at[pl.ds(r, TA), :], xsems.at[i])

    cp["c"].start()
    x_copy(0).start()
    cp["wmod0"].start()

    cp["c"].wait()
    cf = c_v[...].astype(f32)
    sc8 = jnp.broadcast_to((cf * jax.nn.sigmoid(cf)).astype(bf16), (8, D))
    x_copy(0).wait()
    cp["wk"].start()
    n0 = _ln(x_v[0:TA // 2, :].astype(f32))
    cp["wmod0"].wait()
    x_copy(1).start()
    x_copy(2).start()
    mod_v[:, 0:2 * D] = jnp.dot(sc8, wmod_v[:, 0:2 * D], preferred_element_type=f32)

    TH = TA // 2

    def a_ln(j, n=None):
        r = pl.multiple_of(j * TH, TH)
        if n is None:
            n = _ln(x_v[pl.ds(r, TH), :].astype(f32))
        h = (n * (1.0 + mod_v[0:1, D:2 * D]) + mod_v[0:1, 0:D]).astype(bf16)
        h_v[pl.ds(r, TH), :] = h
        return h

    def a_k(j, h):
        kk = jnp.dot(h, wqkv_v[:, D:2 * D], preferred_element_type=f32)
        k_v[pl.ds(pl.multiple_of(j * (TH // 2), TH // 2), TH // 2), :] = pltpu.bitcast(kk.astype(bf16), u32)
        kf_v[pl.ds(pl.multiple_of(j * TH, TH), TH), :] = kk

    h0 = a_ln(0, n0)
    cp["wk"].wait()

    def phase_a1(i, h):
        @pl.when(i + 3 < NA)
        def _():
            x_copy(i + 3).start()

        @pl.when(i == 3)
        def _():
            cp["wq"].start()
            cp["wv"].start()
        x_copy(i + 1).wait()
        hb = a_ln(2 * i + 1)
        a_k(2 * i, h)
        hn = a_ln(2 * i + 2)
        a_k(2 * i + 1, hb)
        return hn
    hl = lax.fori_loop(0, NA - 1, phase_a1, h0)
    cp["wq"].wait()
    cp["wv"].wait()
    for name in ("wmod1", "bsp", "wo", "win", "wout", "wsp"):
        cp[name].start()
    hb = a_ln(2 * NA - 1)
    a_k(2 * NA - 2, hl)
    a_k(2 * NA - 1, hb)
    wqT_v[...] = wqkv_v[:, 0:D].T
    wvT_v[...] = wqkv_v[:, 2 * D:3 * D].T

    def phase_a2(i, vm):
        r = pl.multiple_of(i * TA2, TA2)
        ht = h_v[pl.ds(r, TA2), :]
        qT = lax.dot_general(wqT_v[...], ht, NT, preferred_element_type=f32) * QSCALE
        qf_v[:, :, pl.ds(r, TA2)] = qT.reshape(H, DH, TA2)
        qT_v[:, pl.ds(r, TA2)] = pltpu.bitcast(qT.astype(bf16), u32)
        vT = lax.dot_general(wvT_v[...], ht, NT, preferred_element_type=f32)
        vT_v[:, pl.ds(r, TA2)] = pltpu.bitcast(vT.astype(bf16), u32)
        rh = pl.multiple_of(i * (TA2 // 2), TA2 // 2)
        for g in range(H // 8):
            kg = k_v[pl.ds(rh, TA2 // 2), g * 128:(g + 1) * 128]
            for j in range(8):
                kr_v[g * 8 + j, pl.ds(rh, TA2 // 2), :] = kg if j == 0 else pltpu.roll(kg, 128 - j * DH, 1)
        va = jnp.abs(vT).reshape(D // 8, 8, TA2).max(axis=0)
        for j in range(TA2 // 128):
            vm = jnp.maximum(vm, va[:, j * 128:(j + 1) * 128])
        return vm
    vmax = lax.fori_loop(0, S // TA2, phase_a2, jnp.zeros((8, 128), f32), unroll=2)
    bad_v[...] = jnp.where(vmax <= V_MAX, 0.0, 1.0)

    def build_k(h, kb):
        gl = pl.multiple_of((h // 8) * 128, 128)
        sh = (128 - (h % 8) * DH) % 128
        kk = jnp.concatenate([kf_v[st + ma + mb:st + ma + mb + v, pl.ds(gl, 128)]
                              for (st, ma, mb, v) in SEGS if v], axis=0)
        kk = pltpu.roll(kk, sh, 1)
        for d in range(DH):
            kb[d] = jnp.broadcast_to(kk[:, d:d + 1], (SV, 128))

    def block(u, hp, hc, p_rd, p_wr, l_rd, l_wr, kb_rd, use_vpu, bad):
        consume = hc is not None
        q0 = u * TQ
        qw = _head(qT_v, hp, q0, TQ)
        l = [None] * NL
        acc = None
        npv = 0
        units = {}

        def ladd(li, t):
            l[li] = t if l[li] is None else l[li] + t

        def put(n, val):
            units[n] = val
            if n ^ 1 in units:
                _p_store(p_wr, u, n // 2, units.pop(n & ~1), units.pop(n | 1))

        if use_vpu:
            qb = [jnp.stack([jnp.broadcast_to(qf_v[hp, d:d + 1, q0:q0 + TQ], (8, TQ)) for d in range(4 * e, 4 * e + 4)])
                  for e in range(DH // 4)]

        def vpu8(o):
            cc = None
            for e in range(DH // 4):
                t = kb_rd[4 * e:4 * e + 4, o:o + 8, :] * qb[e]
                cc = t if cc is None else cc + t
            return jnp.exp2((cc[0] + cc[1]) + (cc[2] + cc[3]))

        def qk(a, b, li):
            kk = pltpu.bitcast(kr_v[hp, a // 2:b // 2, :], bf16)[:, 0:DH]
            p = jnp.exp2(jnp.dot(kk, qw, preferred_element_type=f32))
            for r in range((b - a) // 16):
                ladd(li, p[r * 16:r * 16 + 8] + p[r * 16 + 8:r * 16 + 16])
            for r in range((b - a) // 16):
                put(a // 16 + r, p[r * 16:(r + 1) * 16])

        for i, (st, ma, mb, v) in enumerate(SEGS):
            end = st + ma + mb + v
            if use_vpu and v:
                la = (2 * i) % NL
                lb = (2 * i + 1) % NL
                e0 = vpu8(i * SEG_V)
                ladd(la, e0)
                qk(st, st + ma, la)
                e1 = vpu8(i * SEG_V + 8)
                ladd(lb, e1)
                put((end - v) // 16, jnp.concatenate([e0, e1], axis=0))
                qk(st + ma, st + ma + mb, lb)
            else:
                qk(st, end, (2 * i) % NL)
            while consume and (npv + 1) * PVK <= end:
                k0 = npv * PVK
                t = jnp.dot(_head(vT_v, hc, k0, PVK), _p_load(p_rd, u, k0, PVK), preferred_element_type=f32)
                acc = t if acc is None else acc + t
                npv += 1
        if consume:
            ls = l_rd[:, q0:q0 + TQ].sum(axis=0, keepdims=True)
            oT_v[pl.ds(pl.multiple_of(hc * DH, DH), DH), q0:q0 + TQ] = (acc * (1.0 / ls)).astype(bf16)
            bad = jnp.where((ls >= L_LO) & (ls <= L_HI), bad, 1.0)
        l_wr[:, q0:q0 + TQ] = sum(l[1:], l[0])
        return bad

    def mod_rest(j):
        c0 = 2 * D + j * 128
        mod_v[:, c0:c0 + 128] = jnp.dot(sc8, wmod_v[:, c0:c0 + 128], preferred_element_type=f32)
        bj = jnp.broadcast_to(bsp_v[...].astype(f32).reshape(1, S)[:, j * 128:(j + 1) * 128], (128, 128))
        bcol_v[j * 128:(j + 1) * 128, :] = bj.T

    def step(h, p_rd, p_wr, l_rd, l_wr, kb_rd, kb_wr, first=False):
        bad = None if first else bad_v[...]
        for u in range(NQ):
            if first:
                mod_rest(u)
            bad = block(u, h + 1, None if first else h, p_rd, p_wr, l_rd, l_wr, kb_rd, not first, bad)
        if not first:
            bad_v[...] = bad
        build_k(jnp.minimum(h + 2, H - 1), kb_wr)

    cp["wmod1"].wait()
    cp["bsp"].wait()
    step(-1, None, p0, None, l0, kb0, kb1, first=True)

    def phase_b(h, carry):
        lax.cond(h % 2 == 0,
                 lambda: step(h, p0, p1, l0, l1, kb1, kb0),
                 lambda: step(h, p1, p0, l1, l0, kb0, kb1))
        return carry
    lax.fori_loop(0, H - 1, phase_b, 0)
    lsl = l1[...].sum(axis=0, keepdims=True)
    badl = jnp.where((lsl >= L_LO) & (lsl <= L_HI), 0.0, 1.0)
    bad = bad_v[...]
    for j in range(NQ):
        bad = jnp.maximum(bad, badl[:, j * TQ:(j + 1) * TQ])

    @pl.when(jnp.max(bad) > 0.0)
    def _():
        def exact(b, carry):
            h = b // (S // TF)
            q0 = pl.multiple_of((b % (S // TF)) * TF, TF)
            ub = (b % (S // TF)) * (TF // TQ)
            qw = _head(qT_v, h, q0, TF)
            mx = jnp.full((8, TF), -jnp.inf, f32)
            for c in range(S // TK):
                kk = pltpu.bitcast(kr_v[h, c * TK // 2:(c + 1) * TK // 2, :], bf16)[:, 0:DH]
                s = jnp.dot(kk, qw, preferred_element_type=f32)
                sf_v[c * TK:(c + 1) * TK, :] = s
                mx = jnp.maximum(mx, s.reshape(TK // 8, 8, TF).max(axis=0))
            m = mx.max(axis=0, keepdims=True)
            l = jnp.zeros((8, TF), f32)
            acc = jnp.zeros((DH, TF), f32)
            for c in range(S // TK):
                p = jnp.exp2(sf_v[c * TK:(c + 1) * TK, :] - m)
                l = l + p.reshape(TK // 8, 8, TF).sum(axis=0)
                for j in range(TF // TQ):
                    for t in range(TK // 32):
                        _p_store(p1, ub + j, c * (TK // 32) + t, p[t * 32:t * 32 + 16, j * TQ:(j + 1) * TQ],
                                 p[t * 32 + 16:t * 32 + 32, j * TQ:(j + 1) * TQ])
                acc = acc + jnp.dot(_head(vT_v, h, c * TK, TK), p.astype(bf16),
                                    preferred_element_type=f32)
            l1[:, pl.ds(q0, TF)] = l
            o = acc / l.sum(axis=0, keepdims=True)
            oT_v[pl.ds(pl.multiple_of(h * DH, DH), DH), pl.ds(q0, TF)] = o.astype(bf16)
            return carry
        lax.fori_loop(0, H * (S // TF), exact, 0)

    cp["wo"].wait()
    cp["win"].wait()

    def c_s1(i):
        r = pl.multiple_of(i * TC, TC)
        y = lax.dot_general(oT_v[:, pl.ds(r, TC)], wo_v[...], TN, preferred_element_type=f32)
        x1 = x_v[pl.ds(r, TC), :].astype(f32) + mod_v[0:1, 2 * D:3 * D] * y
        x1_v[pl.ds(r, TC), :] = x1
        return (_ln(x1) * (1.0 + mod_v[0:1, 4 * D:5 * D]) + mod_v[0:1, 3 * D:4 * D]).astype(bf16)

    def c_z2(i, h2):
        r = pl.multiple_of(i * TC, TC)
        for a in range(0, TC, TC // 2):
            z2 = _gelu(jnp.dot(h2[a:a + TC // 2], win_v[:, FH:F], preferred_element_type=f32))
            z2_v[pl.ds(r + a, TC // 2), :] = _ln(z2).astype(bf16)

    def c_z1(i, h2):
        r = pl.multiple_of(i * TC, TC)
        z1_v[pl.ds(r, TC), :] = jnp.dot(h2, win_v[:, 0:FH], preferred_element_type=f32).astype(bf16)

    def last_pv(u):
        q0 = u * TQ if isinstance(u, int) else pl.multiple_of(u * TQ, TQ)
        acc = None
        for c in range(S // PVK):
            k0 = c * PVK
            t = jnp.dot(_head(vT_v, H - 1, k0, PVK), _p_load(p1, u, k0, PVK), preferred_element_type=f32)
            acc = t if acc is None else acc + t
        ls = l1[:, pl.ds(q0, TQ)].sum(axis=0, keepdims=True)
        oT_v[(H - 1) * DH:H * DH, pl.ds(q0, TQ)] = (acc * (1.0 / ls)).astype(bf16)

    last_pv(0)
    last_pv(1)
    h20 = c_s1(0)
    for u in range(2, NPRE):
        last_pv(u)

    def phase_c(i, h2):
        c_z2(i, h2)
        hn = c_s1(i + 1)
        c_z1(i, h2)
        last_pv(jnp.minimum(NPRE + i, NQ - 1))
        return hn
    h2 = lax.fori_loop(0, S // TC - 1, phase_c, h20)
    c_z2(S // TC - 1, h2)
    c_z1(S // TC - 1, h2)

    cp["wsp"].wait()
    cp["wout"].wait()

    TO = TD // 2

    def out_copy(j):
        r = pl.multiple_of(j * TO, TO)
        return pltpu.make_async_copy(out_v.at[pl.ds(r, TO), :], out_hbm.at[pl.ds(r, TO), :], osems.at[j])

    def phase_d(i, carry):
        r = pl.multiple_of(i * TD, TD)
        g = jnp.dot(wsp_v[pl.ds(r, TD), :], z2_v[...], preferred_element_type=f32)
        g = g + jnp.concatenate([bcol_v[pl.ds(r, TD), :]] * (FH // 128), axis=1)
        u = (_gelu(z1_v[pl.ds(r, TD), :].astype(f32)) * g).astype(bf16)
        for a in range(2):
            ra = pl.multiple_of(r + a * TO, TO)
            y2 = jnp.dot(u[a * TO:(a + 1) * TO], wout_v[...], preferred_element_type=f32)
            out_v[pl.ds(ra, TO), :] = (x1_v[pl.ds(ra, TO), :] + mod_v[0:1, 5 * D:6 * D] * y2).astype(bf16)
            out_copy(2 * i + a).start()
        return carry
    lax.fori_loop(0, S // TD, phase_d, 0, unroll=2)
    for j in range(S // TO):
        out_copy(j).wait()


@jax.jit
def pallas_adaLN_cond__softmax_full_mha__mixer_gmlp__prompt_kernel(
    A_x: jax.Array,
    A_wqkv: jax.Array,
    A_wo: jax.Array,
    B_x: jax.Array,
    B_w_in: jax.Array,
    B_w_sp: jax.Array,
    B_b_sp: jax.Array,
    B_w_out: jax.Array,
    c: jax.Array,
    w_mod: jax.Array,
):
    del B_x
    any_spec = pl.BlockSpec(memory_space=pl.ANY)
    out = pl.pallas_call(
        _kernel,
        out_shape=jax.ShapeDtypeStruct((S, D), bf16),
        in_specs=[any_spec] * 9,
        out_specs=any_spec,
        scratch_shapes=[
            pltpu.VMEM((S, D), bf16),
            pltpu.VMEM((D, 3 * D), bf16),
            pltpu.VMEM((D, D), bf16),
            pltpu.VMEM((D, F), bf16),
            pltpu.VMEM((S, S), bf16),
            pltpu.VMEM((FH, D), bf16),
            pltpu.VMEM((D, 6 * D), bf16),
            pltpu.VMEM((D, D), bf16),
            pltpu.VMEM((D, D), bf16),
            pltpu.VMEM((S, D), bf16),
            pltpu.VMEM((S // 2, D), u32),
            pltpu.VMEM((S, D), f32),
            pltpu.VMEM((D // 2, S), u32),
            pltpu.VMEM((H, DH, S), f32),
            pltpu.VMEM((D // 2, S), u32),
            pltpu.VMEM((D, S), bf16),
            pltpu.VMEM((DH, SV, 128), f32),
            pltpu.VMEM((DH, SV, 128), f32),
            pltpu.VMEM((H, S // 2, 128), u32),
            pltpu.VMEM((NQ * S // 4, 2 * TQ), u32),
            pltpu.VMEM((NQ * S // 4, 2 * TQ), u32),
            pltpu.VMEM((8, S), f32),
            pltpu.VMEM((8, S), f32),
            pltpu.VMEM((8, TQ), f32),
            pltpu.VMEM((S, TF), f32),
            pltpu.VMEM((S, D), f32),
            pltpu.VMEM((S, FH), bf16),
            pltpu.VMEM((S, FH), bf16),
            pltpu.VMEM((S, 128), f32),
            pltpu.VMEM((8, 6 * D), f32),
            pltpu.VMEM((S, D), bf16),
            pltpu.VMEM((S,), bf16),
            pltpu.VMEM((1, D), bf16),
            pltpu.SemaphoreType.DMA((11,)),
            pltpu.SemaphoreType.DMA((NA,)),
            pltpu.SemaphoreType.DMA((2 * S // TD,)),
        ],
        compiler_params=pltpu.CompilerParams(vmem_limit_bytes=120 * 2 ** 20),
    )(A_x.reshape(S, D), A_wqkv, A_wo, B_w_in, B_w_sp, B_b_sp, B_w_out, c, w_mod)
    return out.reshape(1, S, D)
```
